```python
import os as _os
_os.environ.setdefault('JAX_PLATFORMS', 'cpu')
import jax
import jax.numpy as jnp

def _softmax(x, axis=-1):
    return jax.nn.softmax(x, axis=axis)

def _gelu(x):
    return jax.nn.gelu(x, approximate=True)

def _silu(x):
    return jax.nn.silu(x)

def _sigmoid(x):
    return jax.nn.sigmoid(x)

def _layernorm(x, axis=-1, eps=1e-05):
    m = jnp.mean(x, axis=axis, keepdims=True)
    v = jnp.var(x, axis=axis, keepdims=True)
    return (x - m) / jnp.sqrt(v + eps)

def _scatter_add(tgt, idx, src, axis=0):
    return tgt.at[idx].add(src)

def _segment_sum(src, seg, n):
    return jax.ops.segment_sum(src, seg, n)

class _Rng:

    def __init__(self, key):
        self._k = key

    def _next(self):
        self._k, sub = jax.random.split(self._k)
        return sub

    def normal(self, shape):
        return jax.random.normal(self._next(), shape, dtype=jnp.bfloat16)

    def randint(self, lo, hi, shape):
        return jax.random.randint(self._next(), shape, lo, hi, dtype=jnp.int32)

    def uniform(self, shape, lo=0.0, hi=1.0):
        return jax.random.uniform(self._next(), shape, jnp.bfloat16, lo, hi)

    def permutation(self, n):
        return jax.random.permutation(self._next(), n)
kernel_name = 'gated_mix__sliding_block__memory_aug_recurrent_mem_tr__prompt'

def setup_inputs():
    _rng = _Rng(jax.random.key(int.from_bytes(__import__("os").urandom(4), "little")))
    _w = lambda a: (lambda t: t.astype(jnp.bfloat16) if jnp.issubdtype(t.dtype, jnp.floating) else t)(jnp.asarray(a))

    def _A_setup():
        B, S, D = (1, 2048, 448)
        return {'x': _w((lambda *s: _rng.normal(s) * 0.05)(B, S, D)), 'wqkv': _w((lambda *s: _rng.normal(s) * 0.8)(D, 3 * D)), 'wo': _w((lambda *s: _rng.normal(s) * 0.05)(D, D))}
    _A_in = _A_setup()

    def _B_setup():
        B, S, Dm = (1, 2048, 448)
        H, Dh = (16, 256)
        M, seg = (8, 32)
        seg = min(seg, S)
        S = S // seg * seg
        return {'x': _w((lambda *s: _rng.normal(s) * 0.05)(B, S, Dm)), 'mem0': _w((lambda *s: _rng.normal(s) * 0.8)(B, M, Dm)), 'Wq': _w((lambda *s: _rng.normal(s) * 3.2)(Dm, H, Dh) * Dm ** (-0.5)), 'Wk': _w((lambda *s: _rng.normal(s) * 3.2)(Dm, H, Dh) * Dm ** (-0.5)), 'Wv': _w((lambda *s: _rng.normal(s) * 0.8)(Dm, H, Dh) * Dm ** (-0.5)), 'Wo': _w((lambda *s: _rng.normal(s) * 0.8)(H, Dh, Dm) * (H * Dh) ** (-0.5)), 'seg_len': seg}
    _B_in = _B_setup()
    return {'A_x': _A_in['x'], 'A_wqkv': _A_in['wqkv'], 'A_wo': _A_in['wo'], 'B_x': _B_in['x'], 'B_mem0': _B_in['mem0'], 'B_Wq': _B_in['Wq'], 'B_Wk': _B_in['Wk'], 'B_Wv': _B_in['Wv'], 'B_Wo': _B_in['Wo'], 'B_seg_len': _B_in['seg_len'], 'gate_w': _w((lambda *s: _rng.normal(s) * 0.05)(448) * 16.0)}

def reference(A_x, A_wqkv, A_wo, B_x, B_mem0, B_Wq, B_Wk, B_Wv, B_Wo, B_seg_len, gate_w):

    def _A_ref(x, wqkv, wo):
        B, S, D = x.shape
        H = 16
        Dh = D // H
        W = 256
        qkv = (lambda x, *d: x.transpose(*d))((x @ wqkv).reshape(B, S, 3, H, Dh), 2, 0, 3, 1, 4)
        q, k, v = (qkv[0], qkv[1], qkv[2])
        scores = jnp.einsum('bhqd,bhkd->bhqk', q, k) * Dh ** (-0.5)
        idx = jnp.arange(S)
        mask = (idx[:, None] - idx[None, :] >= 0) & (idx[:, None] - idx[None, :] < W)
        scores = jnp.where(mask[None, None], scores, -1000000000.0)
        p = _softmax(scores, axis=-1)
        o = jnp.einsum('bhqk,bhkd->bhqd', p, v)
        return (lambda x, *d: x.transpose(*d))(o, 0, 2, 1, 3).reshape(B, S, D) @ wo

    def _B_ref(x, mem0, Wq, Wk, Wv, Wo, seg_len):
        B, S, Dm = x.shape
        H, Dh = (Wq.shape[1], Wq.shape[2])
        M = mem0.shape[1]
        scale = Dh ** (-0.5)
        n_seg = S // seg_len
        L = M + seg_len
        idx = jnp.arange(L)
        mask = (idx[:, None] < M) | (idx[:, None] >= idx[None, :])
        mem = mem0
        outs = []
        for s in range(n_seg):
            xs = x[:, s * seg_len:(s + 1) * seg_len, :].copy()
            h = jnp.concatenate([mem, xs], axis=1)
            q = jnp.einsum('btd,dhe->bhte', h, Wq)
            k = jnp.einsum('btd,dhe->bhte', h, Wk)
            v = jnp.einsum('btd,dhe->bhte', h, Wv)
            scores = jnp.einsum('bhqe,bhke->bhqk', q, k) * scale
            scores = jnp.where(mask[None, None], scores, -1000000000.0)
            p = _softmax(scores, axis=-1)
            o = jnp.einsum('bhqk,bhke->bhqe', p, v)
            o = jnp.einsum('bhte,hed->btd', o, Wo)
            mem = o[:, :M, :].copy()
            outs.append(o[:, M:, :])
        return jnp.concatenate(outs, axis=1)
    x = A_x
    g = _sigmoid((x * gate_w).sum(-1, keepdims=True))
    a = _A_ref(x, A_wqkv, A_wo)
    b = _B_ref(x, B_mem0, B_Wq, B_Wk, B_Wv, B_Wo, B_seg_len)
    return g * a + (1 - g) * b
```

```python
import functools
import math

import jax
import jax.numpy as jnp
import numpy as np
from jax import lax
from jax.experimental import pallas as pl
from jax.experimental.pallas import tpu as pltpu

F32 = jnp.float32
BF16 = jnp.bfloat16
U32 = jnp.uint32
LOG2E = math.log2(math.e)
NEG = -1000000000.0

NN = (((1,), (0,)), ((), ()))
NT = (((1,), (1,)), ((), ()))

ORDER = "sa0 sa1 sa2 sa3 t0 t1 pa0 t2 pa1 t3 pa2 t4 pa3 t5 t6 t7 v0 sb v1 v2 v3 v4 v5 v6 v7 fin pb"
UNROLL = 1


def _dot(a, b, dims=NN):
    return lax.dot_general(a, b, dims, preferred_element_type=F32)


def _to_u32(x_bf16):
    return pltpu.bitcast(x_bf16, U32)


def _to_bf16(x_u32):
    return pltpu.bitcast(x_u32, BF16)


def _iota(shape, dim):
    return lax.broadcasted_iota(jnp.int32, shape, dim)


def _group8_allreduce(x, op):
    lane = _iota(x.shape, 1)
    for d in (1, 2, 4):
        up = pltpu.roll(x, 128 - d, 1)
        dn = pltpu.roll(x, d, 1)
        x = op(x, jnp.where((lane & d) == 0, up, dn))
    return x


def _kernel(xt_hbm, wqkv_hbm, wo_hbm, mem0_hbm, wq_hbm, wk_hbm, wv_hbm, bwo_hbm, gw_hbm,
            out_hbm,
            xt_v, wqkv_v, wo_v, mem0_v, gw_v, wq_v, wk_v, wv_v, bwo_v,
            wq_s, wk_s, wv_s, wt_s, wb_s,
            wa_s, wot_s, xn_s, g_s, ka_s, qt_s, vt_s, oa_s, b_s, bt_s, out_v,
            ts_s, vs_s, pa_s,
            sems, osem):
    S, D = 2048, 448
    NQB = S // 128

    copies = dict(
        wqkv=pltpu.make_async_copy(wqkv_hbm, wqkv_v, sems.at[0]),
        gw=pltpu.make_async_copy(gw_hbm, gw_v, sems.at[8]),
        x=pltpu.make_async_copy(xt_hbm.at[0], xt_v, sems.at[1]),
        wq=pltpu.make_async_copy(wq_hbm, wq_v, sems.at[2]),
        wk=pltpu.make_async_copy(wk_hbm, wk_v, sems.at[3]),
        bwo=pltpu.make_async_copy(bwo_hbm, bwo_v, sems.at[4]),
        wv=pltpu.make_async_copy(wv_hbm, wv_v, sems.at[5]),
        wo=pltpu.make_async_copy(wo_hbm, wo_v, sems.at[6]),
        mem0=pltpu.make_async_copy(mem0_hbm.at[0], mem0_v, sems.at[7]),
    )
    for c in copies.values():
        c.start()

    lane128 = _iota((128, 128), 1)
    kpad = _to_u32(jnp.where(lane128 == 127, NEG, 0.0).astype(BF16))
    for hg in range(4):
        ka_s[hg, 0:64, :] = kpad
        ka_s[hg, 64:128, :] = kpad
        for i in range(2):
            for r in range(0, 112, 56):
                vt_s[hg, i, r:r + 56, :] = jnp.zeros((56, 128), F32)
    for r in range(0, 224, 56):
        oa_s[1, r:r + 56, :] = jnp.zeros((56, 128), U32)
    for r in range(0, 128, 16):
        b_s[1, r:r + 16, :] = jnp.zeros((16, 512), F32)

    copies["wqkv"].wait()
    for c in range(0, 3 * D, 128):
        n = min(128, 3 * D - c)
        wa_s[c // 2:(c + n) // 2, :] = _to_u32(wqkv_v[:, c:c + n].astype(F32).T.astype(BF16))
    copies["gw"].wait()
    gw = gw_v[...].astype(F32).reshape(1, D)
    wa_s[3 * D // 2:3 * D // 2 + 8, :] = _to_u32(jnp.broadcast_to(gw, (16, D)).astype(BF16))

    copies["x"].wait()
    qscale = 28.0 ** -0.5 * LOG2E

    def proj_a(qb, carry):
        xt = xt_v[:, pl.ds(pl.multiple_of(qb * 128, 128), 128)]
        y = _dot(_to_bf16(wa_s[...]), xt)
        xf = xt.astype(F32)
        xn_s[pl.ds(pl.multiple_of(qb * 128, 128), 128), :] = jnp.concatenate([xf, xf[384:448]], axis=0).T
        row = pl.multiple_of(128 + qb * 64, 64)
        for hg in range(4):
            q = y[112 * hg:112 * (hg + 1)] * qscale
            qt_s[qb * 4 + hg] = _to_u32(q.astype(BF16))
            k = jnp.concatenate([y[D + 112 * hg:D + 112 * (hg + 1)], jnp.zeros((16, 128), F32)], axis=0)
            ka_s[hg, pl.ds(row, 64), :] = _to_u32(k.T.astype(BF16))
            vt_s[hg, qb + 2] = y[2 * D + 112 * hg:2 * D + 112 * (hg + 1)]
        g_s[qb] = jax.nn.sigmoid(y[3 * D:3 * D + 8])
        return carry

    lax.fori_loop(0, NQB, proj_a, 0)

    def deinterleave(src, dst):
        def body(i, carry):
            for j in range(7):
                r = i * 7 + j
                for c in range(2):
                    v = _to_u32(src[pl.ds(pl.multiple_of(r * 128, 128), 128), c * 128:(c + 1) * 128])
                    v = jnp.swapaxes(v.reshape(8, 8, 128), 0, 1)
                    dst[:, pl.ds(pl.multiple_of(r * 8, 8), 8), c * 128:(c + 1) * 128] = v
            return carry
        lax.fori_loop(0, 8, body, 0)

    def split_pair(w):
        lo = pltpu.bitcast(w << 16, F32)
        hi = pltpu.bitcast(w & jnp.uint32(0xFFFF0000), F32)
        return lo, hi

    lane_lo = _iota((D, 128), 1) < 64

    def merge(dst, p, la, lb, ra, rb, scale):
        sc = (lambda y: y) if scale is None else (lambda y: y * scale)
        dst[p, :, 0:384] = _to_u32(sc(_dot(la, ra[0:384], NT)).astype(BF16))
        dst[p, :, 384:768] = _to_u32(sc(_dot(lb, rb[0:384], NT)).astype(BF16))
        r3 = jnp.concatenate([ra[384:448], rb[384:448]], axis=0)
        dst[p, :, 768:896] = _to_u32(sc(jnp.where(lane_lo, _dot(la, r3, NT), _dot(lb, r3, NT))).astype(BF16))

    copies["wq"].wait()
    deinterleave(wq_v, wq_s)
    copies["wk"].wait()
    deinterleave(wk_v, wk_s)

    def merge_qk(p, carry):
        qa, qb = split_pair(wq_s[p])
        ka, kb = split_pair(wk_s[p])
        merge(wt_s, p, ka, kb, qa.astype(BF16), qb.astype(BF16), 256.0 ** -0.5 * LOG2E)
        return carry

    lax.fori_loop(0, 8, merge_qk, 0)

    copies["wv"].wait()
    deinterleave(wv_v, wv_s)
    copies["bwo"].wait()

    def merge_vo(p, carry):
        va, vb = split_pair(wv_s[p])
        merge(wb_s, p, va, vb, bwo_v[2 * p], bwo_v[2 * p + 1], None)
        return carry

    lax.fori_loop(0, 8, merge_vo, 0)

    copies["wo"].wait()
    for c in range(0, D, 128):
        n = min(128, D - c)
        wot_s[c // 2:(c + n) // 2, :] = _to_u32(wo_v[:, c:c + n].astype(F32).T.astype(BF16))
    copies["mem0"].wait()

    def stack_heads(dst, p, y):
        lo = _iota((8, 128), 1) < 64
        for t in range(5):
            yt = y[8 * t:8 * (t + 1)]
            y3 = yt[:, 768:896]
            ra = jnp.concatenate([yt[:, 0:384], jnp.where(lo, y3, 0.0)], axis=1)
            rb = jnp.concatenate([yt[:, 384:768], jnp.where(lo, 0.0, y3)], axis=1)
            dst[t, 8 * p:8 * (p + 1), :] = _to_u32(jnp.concatenate([ra, rb], axis=0).astype(BF16))

    def finalize(slot, hg, blk):
        r0 = hg * 112
        c0 = hg * 128 if isinstance(hg, int) else pl.multiple_of(hg * 128, 128)
        bt_s[pl.ds(c0, 128), :] = b_s[slot, :, pl.ds(c0, 128)].T
        al = (lambda v, n: v) if isinstance(hg, int) else pl.multiple_of
        a = _dot(_to_bf16(wot_s[pl.ds(al(hg * 56, 8), 56), :]), _to_bf16(oa_s[slot]))
        b = bt_s[pl.ds(al(r0, 16), 112), :]
        g = jnp.broadcast_to(g_s[blk][0:1], (112, 128))
        out_v[blk, pl.ds(al(r0, 16), 112), :] = (g * a + (1.0 - g) * b).astype(BF16)

    def out_copy(blk):
        col = blk * 128 if isinstance(blk, int) else pl.multiple_of(blk * 128, 128)
        return pltpu.make_async_copy(out_v.at[blk], out_hbm.at[0, :, pl.ds(col, 128)], osem)

    def step(s, mem):
        qb = s // 4
        hg = s % 4
        slot = qb % 2
        st = {}

        xs = xn_s[pl.ds(pl.multiple_of(s * 32, 32), 32), :]
        h = jnp.concatenate([mem, xs], axis=0)
        hk = h[:, 0:D]

        def op_t(p):
            stack_heads(ts_s, p, _dot(hk, _to_bf16(wt_s[p])))

        def op_v(p):
            stack_heads(vs_s, p, _dot(hk, _to_bf16(wb_s[p])))

        def op_sb():
            sc = []
            for t in range(5):
                q = h if t <= 1 else jnp.concatenate([h[0:8], h[8 * t:40]], axis=0)
                y = _dot(q, _to_bf16(ts_s[t]), NT)
                rows = list(range(5)) if t <= 1 else [0] + list(range(t, 5))
                sc.append({i: y[8 * n:8 * (n + 1)] for n, i in enumerate(rows)})
            causal = (_iota((8, 128), 1) & 7) <= _iota((8, 128), 0)
            for i in range(1, 5):
                sc[i][i] = jnp.where(causal, sc[i][i], NEG)
            mx = [functools.reduce(jnp.maximum, [sc[t][i] for t in range(5) if i in sc[t]]) for i in range(5)]
            mx = _group8_allreduce(jnp.concatenate(mx, axis=0), jnp.maximum)
            for t in range(5):
                for i in sc[t]:
                    sc[t][i] = jnp.exp2(sc[t][i] - mx[8 * i:8 * (i + 1)])
            ls = [functools.reduce(jnp.add, [sc[t][i] for t in range(5) if i in sc[t]]) for i in range(5)]
            inv = 1.0 / _group8_allreduce(jnp.concatenate(ls, axis=0), jnp.add)
            st["p"] = [{i: sc[t][i] * inv[8 * i:8 * (i + 1)] for i in sc[t]} for t in range(5)]

        def op_pb():
            acc = [None] * 5
            for t in range(5):
                rows = sorted(st["p"][t])
                y = _dot(jnp.concatenate([st["p"][t][i] for i in rows], axis=0), _to_bf16(vs_s[t]))
                for n, i in enumerate(rows):
                    yi = y[8 * n:8 * (n + 1)]
                    acc[i] = yi if acc[i] is None else acc[i] + yi
            o = jnp.concatenate(acc, axis=0)
            o3 = o[:, 384:512]
            o = jnp.concatenate([o[:, 0:384], o3 + pltpu.roll(o3, 64, 1)], axis=1)
            b_s[slot, pl.ds(pl.multiple_of(hg * 32, 32), 32), :] = o[8:40]
            st["mem"] = o[0:8]

        def op_sa(j):
            tri = _iota((128, 128), 0) <= _iota((128, 128), 1)
            r112 = _iota((112, 128), 0)
            kw = _to_bf16(ka_s[hg, pl.ds(pl.multiple_of(qb * 64, 64), 192), :])
            qt = _to_bf16(qt_s[s]).astype(F32)
            one = jnp.where(_iota((16, 128), 0) == 15, 1.0, 0.0).astype(BF16)
            qj = jnp.where((r112 >= 28 * j) & (r112 < 28 * (j + 1)), qt, 0.0).astype(BF16)
            sa = _dot(kw, jnp.concatenate([qj, one], axis=0))
            sm = jnp.where(tri, sa[256:384], sa[0:128])
            sc = sa[128:256]
            m = jnp.max(jnp.maximum(sm, sc), axis=0, keepdims=True)
            pm = jnp.exp2(sm - m)
            pc = jnp.exp2(sc - m)
            st["l", j] = jnp.sum(pm + pc, axis=0, keepdims=True)
            p = jnp.concatenate([jnp.where(tri, 0.0, pm), pc, jnp.where(tri, pm, 0.0)], axis=0)
            pa_s[j] = _to_u32(p.astype(BF16))

        def op_pa(j):
            w0 = (0, 24, 56, 80)[j]
            v = jnp.concatenate([vt_s[hg, qb + i, w0:w0 + 32, :] for i in range(3)], axis=1)
            st["o", j] = _dot(v, _to_bf16(pa_s[j])) * (1.0 / st["l", j])
            if all(("o", i) in st for i in range(4)):
                o = [st["o", i] for i in range(4)]
                first4 = _iota((8, 128), 0) < 4
                ot = jnp.concatenate([
                    o[0][0:24], jnp.where(first4, o[0][24:32], o[1][0:8]), o[1][8:32],
                    o[2][0:24], jnp.where(first4, o[2][24:32], o[3][0:8]), o[3][8:32]], axis=0)
                oa_s[slot, pl.ds(pl.multiple_of(hg * 56, 8), 56), :] = _to_u32(ot.astype(BF16))

        def op_fin():
            finalize(1 - slot, hg, jnp.maximum(qb - 1, 0))

        ops = dict(t=op_t, v=op_v, sb=op_sb, pb=op_pb, sa=op_sa, pa=op_pa, fin=op_fin)
        for name in ORDER.split():
            if name[-1].isdigit():
                ops[name[:-1]](int(name[-1]))
            else:
                ops[name]()
        return st["mem"]

    def body(i, mem):
        s0 = i * UNROLL

        @pl.when((s0 >= 8) & (s0 % 4 == 0))
        def _():
            out_copy(s0 // 4 - 2).start()

        for u in range(UNROLL):
            mem = step(s0 + u, mem)
        return mem

    m0 = mem0_v[...].astype(F32)
    lax.fori_loop(0, 64 // UNROLL, body, jnp.concatenate([m0, m0[:, 384:448]], axis=1))

    out_copy(NQB - 2).start()
    for hg in range(4):
        finalize(1, hg, NQB - 1)
    out_copy(NQB - 1).start()
    for blk in range(NQB):
        out_copy(blk).wait()


@functools.partial(jax.jit, static_argnames=("B_seg_len",))
def pallas_gated_mix__sliding_block__memory_aug_recurrent_mem_tr__prompt_kernel(
        A_x, A_wqkv, A_wo, B_x, B_mem0, B_Wq, B_Wk, B_Wv, B_Wo, B_seg_len, gate_w):
    del B_x
    assert A_x.shape == (1, 2048, 448) and B_Wq.shape == (448, 16, 256)
    assert B_mem0.shape == (1, 8, 448) and int(B_seg_len) == 32
    S, D = 2048, 448
    flat = lambda w: w.reshape(D * 16, 256)
    hbm = pl.BlockSpec(memory_space=pltpu.HBM)
    vmem = pltpu.VMEM
    out_t = pl.pallas_call(
        _kernel,
        out_shape=jax.ShapeDtypeStruct((1, D, S), BF16),
        in_specs=[hbm] * 9,
        out_specs=hbm,
        scratch_shapes=[
            vmem((D, S), BF16), vmem((D, 3 * D), BF16), vmem((D, D), BF16), vmem((8, D), BF16),
            vmem((D,), BF16),
            vmem((D * 16, 256), BF16), vmem((D * 16, 256), BF16), vmem((D * 16, 256), BF16),
            vmem((16, D, 256), BF16),
            vmem((8, D, 256), U32), vmem((8, D, 256), U32), vmem((8, D, 256), U32),
            vmem((8, D // 2, 896), U32), vmem((8, D // 2, 896), U32),
            vmem((3 * D // 2 + 8, D), U32), vmem((D // 2, D), U32), vmem((S, 512), F32),
            vmem((16, 8, 128), F32),
            vmem((4, (S + 256) // 2, 128), U32), vmem((64, 56, 128), U32),
            vmem((4, 18, 112, 128), F32),
            vmem((2, D // 2, 128), U32), vmem((2, 128, 512), F32), vmem((512, 128), F32),
            vmem((16, D, 128), BF16),
            vmem((5, 64, 512), U32), vmem((5, 64, 512), U32), vmem((4, 192, 128), U32),
            pltpu.SemaphoreType.DMA((9,)), pltpu.SemaphoreType.DMA(()),
        ],
        compiler_params=pltpu.CompilerParams(vmem_limit_bytes=100 * 2**20),
        name="mykern",
    )(A_x.transpose(0, 2, 1), A_wqkv, A_wo, B_mem0, flat(B_Wq), flat(B_Wk), flat(B_Wv),
      B_Wo.transpose(0, 2, 1), gate_w)
    return out_t.transpose(0, 2, 1)
```

```python
import functools
import math

import jax
import jax.numpy as jnp
import numpy as np
from jax import lax
from jax.experimental import pallas as pl
from jax.experimental.pallas import tpu as pltpu

F32 = jnp.float32
BF16 = jnp.bfloat16
U32 = jnp.uint32
LOG2E = math.log2(math.e)
NEG = -1000000000.0

NN = (((1,), (0,)), ((), ()))
NT = (((1,), (1,)), ((), ()))

ORDER = ("t00 t10 t20 t30 t01 t11 tr t21 t02 t31 t22 t33 t32 t03 t13 t23 v00 t12 v10 sa0 sb0 sb1 sa1 v20 sa3 "
         "sb2 v30 sa2 sb3 v01 sb4 v11 v31 v03 rg0 rg1 rg3 v13 v23 v33 v02 rg2 v22 v21 v12 v32 "
         "pb1 pb0 pa3 pa1 pb3 pb2 pa2 fin pa0")
LAST = None
UNROLL = 4
NOXP = False
NOROLL = False
NOBC = False
NOPRO = False
MINSLAB = 5
SACUT = [0, 40, 72, 112, 144]
P1 = 2
P2 = 2
AHEAD = 2
MU = 1
NODMA = False
SCOPES = False


def _scope(name):
    import contextlib
    return jax.named_scope(name) if SCOPES else contextlib.nullcontext()


def _dot(a, b, dims=NN):
    return lax.dot_general(a, b, dims, preferred_element_type=F32)


def _to_u32(x_bf16):
    return pltpu.bitcast(x_bf16, U32)


def _to_bf16(x_u32):
    return pltpu.bitcast(x_u32, BF16)


def _iota(shape, dim):
    return lax.broadcasted_iota(jnp.int32, shape, dim)


def _al(v, n):
    return v if isinstance(v, int) else pl.multiple_of(v, n)


def _group8_allreduce(x, op):
    if NOROLL:
        return x
    lane = _iota(x.shape, 1)
    for d in (1, 2, 4):
        up = pltpu.roll(x, 128 - d, 1)
        dn = pltpu.roll(x, d, 1)
        x = op(x, jnp.where((lane & d) == 0, up, dn))
    return x


HEAD_WIN = (0, 24, 56, 80)


def _join_heads(w):
    first4 = _iota((8, w[0].shape[1]), 0) < 4
    return jnp.concatenate([
        w[0][0:24], jnp.where(first4, w[0][24:32], w[1][0:8]), w[1][8:32],
        w[2][0:24], jnp.where(first4, w[2][24:32], w[3][0:8]), w[3][8:32]], axis=0)


def _regroup(z):
    lane = _iota(z[0].shape, 1)
    y = [jnp.where((lane & 32) != 0, z[(k + 1) % 4], z[k]) for k in range(4)]
    x = [jnp.where((lane & 64) != 0, y[(k + 2) % 4], y[k]) for k in range(4)]
    return [x[(-j) % 4] for j in range(4)]


WQ, WK = 0, 7168
KA = 14336
QT = 18944
VT = 22528
WT, WV = 0, 12544


def _loop(n, body, unroll):
    if unroll == n:
        for i in range(n):
            body(i, 0)
    else:
        lax.fori_loop(0, n, body, 0, unroll=max(unroll, 1))


def _when(cond):
    if isinstance(cond, bool):
        return lambda f: f() if cond else None
    return pl.when(cond)


def _kernel(xt_hbm, wqkv_hbm, wo_hbm, mem0_hbm, wq_hbm, wk_hbm, wv_hbm, bwo_hbm, gw_hbm,
            out_hbm,
            xt_v, wqkv_v, wo_v, mem0_v, gw_v, wq_v, wk_v, wv_v, bwo_v,
            ar1, ar2, ar3,
            wa_s, wat_s, gw_s, wot_s, xn_s, g_s, oa_s, b_s, bt_s, out_v,
            ts_s, vs_s, pa_s, pz_s,
            sems, wsem, osem):
    S, D = 2048, 448
    NQB = S // 128

    small = dict(
        wqkv=pltpu.make_async_copy(wqkv_hbm, wqkv_v, sems.at[0]),
        gw=pltpu.make_async_copy(gw_hbm, gw_v, sems.at[1]),
        wo=pltpu.make_async_copy(wo_hbm, wo_v, sems.at[2]),
        mem0=pltpu.make_async_copy(mem0_hbm.at[0], mem0_v, sems.at[3]),
    )

    def x_copy(i):
        cols = pl.ds(_al(i * 512, 512), 512)
        return pltpu.make_async_copy(xt_hbm.at[0, :, cols], xt_v.at[:, cols], sems.at[4 + i])

    def w_copy(which, i):
        src, dst = ((wq_hbm, wq_v), (wk_hbm, wk_v), (wv_hbm, wv_v))[which]
        rows = pl.ds(_al(i * 896, 896), 896)
        return pltpu.make_async_copy(src.at[rows], dst.at[rows], wsem.at[8 * which + i])

    def bwo_copy(q):
        heads = pl.ds(4 * q, 4)
        return pltpu.make_async_copy(bwo_hbm.at[heads], bwo_v.at[heads], wsem.at[24 + q])

    small["wqkv"].start()
    small["gw"].start()
    x_copy(0).start()

    lane128 = _iota((128, 128), 1)
    kpad = _to_u32(jnp.where(lane128 == 127, NEG, 0.0).astype(BF16))
    for hg in range(4):
        ar1[KA + 1152 * hg:KA + 1152 * hg + 64, :] = kpad
        ar1[KA + 1152 * hg + 64:KA + 1152 * hg + 128, :] = kpad
        for r in range(0, 224, 56):
            ar1[VT + 2016 * hg + r:VT + 2016 * hg + r + 56, :] = jnp.zeros((56, 128), U32)
    for r in range(0, 224, 56):
        oa_s[1, r:r + 56, :] = jnp.zeros((56, 128), U32)
    for r in range(0, 128, 16):
        b_s[1, r:r + 16, :] = jnp.zeros((16, 512), F32)

    with _scope("wqkv_wait"):
        small["wqkv"].wait()
    for i in range(1, 4):
        x_copy(i).start()
    for i in range(AHEAD):
        w_copy(0, i).start()
        w_copy(1, i).start()
    for c in range(0, 3 * D, 128):
        n = min(128, 3 * D - c)
        w = wqkv_v[:, c:c + n].astype(F32)
        wat_s[c:c + n, :] = jnp.concatenate([w, w[384:448]], axis=0).T
    for part in range(3):
        for r in range(0, 224, 32):
            u = wat_s[D * part + r:D * part + r + 32, :]
            v = wat_s[D * part + 224 + r:D * part + 224 + r + 32, :]
            lo = _iota((32, 128), 1) < 64
            dst = slice((224 * part + r) // 2, (224 * part + r) // 2 + 16)
            u2, u3, v2, v3 = u[:, 256:384], u[:, 384:512], v[:, 256:384], v[:, 384:512]
            w = jnp.concatenate([u[:, 0:256], jnp.where(lo, u2, u2 - v2),
                                 v[:, 0:256], jnp.where(lo, v2, v3 - u3),
                                 jnp.where(lo, u3, v2)], axis=1)
            wa_s[dst, :] = _to_u32(w.astype(BF16))
    small["gw"].wait()
    gw = jnp.broadcast_to(gw_v[...].astype(F32).reshape(1, D), (16, D))
    gw_s[...] = _to_u32(gw.astype(BF16))

    qscale = 28.0 ** -0.5 * LOG2E

    def proj_a(qb, extra=lambda k: None):
        if NOPRO:
            return
        xt = xt_v[:, pl.ds(_al(qb * 128, 128), 128)]
        x1 = xt[0:384]
        x2 = jnp.concatenate([xt[0:320], xt[384:448]], axis=0)
        x3 = jnp.concatenate([xt[384:448], xt[320:384]], axis=0)

        def piece(k, g):
            rows = slice(112 * k + 56 * g, 112 * k + 56 * (g + 1))
            shared = _dot(_to_bf16(wa_s[rows, 768:896]), x3)
            return ((g, _dot(_to_bf16(wa_s[rows, 0:384]), x1) + shared),
                    (g + 2, _dot(_to_bf16(wa_s[rows, 384:768]), x2) + shared))

        xf = xt.astype(F32)
        xn_s[pl.ds(_al(qb * 128, 128), 128), :] = jnp.concatenate([xf, xf[384:448]], axis=0).T
        for g in range(2):
            for hg, y in piece(1, g):
                k = jnp.concatenate([y, jnp.zeros((16, 128), F32)], axis=0)
                ar1[pl.ds(_al(KA + 1152 * hg + 128 + qb * 64, 64), 64), :] = _to_u32(k.T.astype(BF16))
            extra(g)
        for g in range(2):
            for hg, y in piece(0, g):
                q = y * qscale
                q = _join_heads([q[0:32]] + [pltpu.roll(q[w:w + 32], 32 * j, 1)
                                             for j, w in enumerate(HEAD_WIN) if j])
                ar1[pl.ds(_al(QT + (qb * 4 + hg) * 56, 8), 56), :] = _to_u32(q.astype(BF16))
            extra(2 + g)
        g_s[qb] = jax.nn.sigmoid(_dot(_to_bf16(gw_s[...]), xt)[0:8])
        for g in range(2):
            for hg, y in piece(2, g):
                ar1[pl.ds(_al(VT + 2016 * hg + (qb + 2) * 112, 16), 112), :] = pltpu.bitcast(y, U32)
            extra(4 + g)

    def deinterleave(src, arena, dst, i, js):
        for j in js:
            r = i * 7 + j
            for c in range(2):
                v = _to_u32(src[pl.ds(_al(r * 128, 128), 128), c * 128:(c + 1) * 128])
                v = jnp.swapaxes(v.reshape(8, 8, 128), 0, 1)
                for p in range(8):
                    arena[pl.ds(_al(dst + (2 * p + c) * D + r * 8, 8), 8), :] = v[p]

    def phase1(i, carry):
        _when(i * P1 % 4 == 0)(lambda: x_copy(i * P1 // 4).wait())
        for u in range(P1):
            proj_a(i * P1 + u)
        for u in range(P1):
            n = i * P1 + u + AHEAD

            @_when(n < 8)
            def _():
                w_copy(0, n).start()
                w_copy(1, n).start()

        return carry

    with _scope('phase1'):
        _loop(8 // P1, phase1, 1)

    def phase2(i, carry):
        _when(i * P2 % 4 == 0)(lambda: x_copy(2 + i * P2 // 4).wait())
        for u in range(P2):
            w_copy(0, i * P2 + u).wait()
            w_copy(1, i * P2 + u).wait()
        for u in range(P2):
            n = i * P2 + u

            def extra(k):
                src, dst = (wq_v, WQ) if k < 3 else (wk_v, WK)
                deinterleave(src, ar1, dst, n, (range(0, 3), range(3, 5), range(5, 7))[k % 3])

            proj_a(8 + n, extra)
        for u in range(P2):
            w_copy(2, i * P2 + u).start()
        return carry

    with _scope('phase2'):
        _loop(8 // P2, phase2, 1)

    def head_rows(arena, base, head4, k, r0=0, n=D):
        p = head4 // 2 + k // 2
        w = jnp.concatenate([arena[pl.ds(_al(base + (2 * p + c) * D + r0, 64), n), :] for c in range(2)], axis=1)
        return pltpu.bitcast(w << 16 if k % 2 == 0 else w & jnp.uint32(0xFFFF0000), F32)

    def merge(dst, q, lhs, rhs, scale, extra=lambda k: None):
        if NOPRO:
            return
        sc = (lambda y: y) if scale is None else (lambda y: y * scale)

        def put(tile, u, v):
            u3 = u[384:448].astype(BF16)
            v2 = v[320:384].astype(BF16)
            w = jnp.concatenate([
                u[0:320].astype(BF16), (u[320:384] - v2.astype(F32)).astype(BF16),
                v[0:320].astype(BF16), (v[384:448] - u3.astype(F32)).astype(BF16),
                u3, v2], axis=0)
            dst[pl.ds(_al((q * 7 + tile) * D, 64), D), :] = _to_u32(w)

        def block(i, c):
            put(3 * i + c, sc(_dot(lhs(i), rhs(i, 128 * c, 128), NT)),
                sc(_dot(lhs(2 + i), rhs(2 + i, 128 * c, 128), NT)))

        block(0, 0)
        extra(0)
        tail = [jnp.concatenate([_dot(rhs(k, 384, 64), lhs(k).astype(BF16), NT) for k in (i, i + 1)], axis=0)
                for i in (0, 2)]
        block(0, 1)
        extra(1)
        put(6, sc(tail[0].T), sc(tail[1].T))
        extra(2)
        block(0, 2)
        extra(3)
        block(1, 0)
        extra(4)
        block(1, 1)
        extra(5)
        block(1, 2)

    def merge_qk(q, carry):
        w_copy(2, 2 * q).wait()
        w_copy(2, 2 * q + 1).wait()

        def extra(k):
            deinterleave(wv_v, ar2, WV, 2 * q + k // 3, (range(0, 3), range(3, 5), range(5, 7))[k % 3])

        merge(ar2, q, lambda k: head_rows(ar1, WK, 4 * q, k),
              lambda k, r0, n: head_rows(ar1, WQ, 4 * q, k, r0, n).astype(BF16), 256.0 ** -0.5 * LOG2E, extra)

        @_when(q < 3)
        def _():
            bwo_copy(q + 1).start()

        return carry

    bwo_copy(0).start()
    small["wo"].start()
    small["mem0"].start()
    with _scope('merge_qk'):
        _loop(4, merge_qk, MU)
    small["wo"].wait()

    def transpose_wo(q):
        c, n = 128 * q, min(128, D - 128 * q)
        wot_s[c // 2:(c + n) // 2, :] = _to_u32(wo_v[:, c:c + n].astype(F32).T.astype(BF16))

    def merge_vo(q, carry):
        bwo_copy(q).wait()
        if MU == 4:
            transpose_wo(q)
        merge(ar3, q, lambda k: head_rows(ar2, WV, 4 * q, k),
              lambda k, r0, n: bwo_v[4 * q + k, r0:r0 + n, :], None)
        return carry

    with _scope('merge_vo'):
        _loop(4, merge_vo, MU)
    if MU < 4:
        for q in range(4):
            transpose_wo(q)

    small["mem0"].wait()

    def transpose_b(slot, hg):
        c0 = _al(hg * 128, 128)
        bt_s[pl.ds(c0, 128), :] = b_s[slot, :, pl.ds(c0, 128)].T

    def finalize(slot, hg, blk):
        a = _dot(_to_bf16(wot_s[pl.ds(_al(hg * 56, 8), 56), :]), _to_bf16(oa_s[slot]))
        b = bt_s[pl.ds(_al(hg * 112, 16), 112), :]
        g = jnp.broadcast_to(g_s[blk][0:1], (112, 128))
        out_v[blk, pl.ds(_al(hg * 112, 16), 112), :] = (g * a + (1.0 - g) * b).astype(BF16)

    def out_copy(blk):
        return pltpu.make_async_copy(out_v.at[blk], out_hbm.at[0, :, pl.ds(_al(blk * 128, 128), 128)], osem)

    def step(qb, hg, mem, last):
        s = qb * 4 + hg
        slot = qb & 1
        st = {}

        xs = xn_s[pl.ds(pl.multiple_of(s * 32, 32), 32), :]
        h = jnp.concatenate([mem, xs], axis=0)
        lo40 = _iota((40, 128), 1) < 64
        lo8 = _iota((8, 128), 1) < 64
        l1 = h[:, 0:384]
        l2 = jnp.concatenate([h[:, 0:256], jnp.where(lo40, h[:, 256:384], h[:, 384:512])], axis=1)
        l3 = jnp.where(lo40, h[:, 384:512], h[:, 256:384])

        def two_tiles(w, q, c):
            o = (q * 7 + c) * D
            shared = _dot(l3, _to_bf16(w[o + 384:o + 448, :]))
            return (_dot(l1, _to_bf16(w[o:o + 192, :])) + shared,
                    _dot(l2, _to_bf16(w[o + 192:o + 384, :])) + shared)

        def project(w, dst, q, c):
            def put(i, u, v):
                for t in range(5):
                    rows = slice(8 * t, 8 * (t + 1))
                    dst[t, c, 32 * q + 16 * i:32 * q + 16 * (i + 1), :] = (
                        jnp.concatenate([u[rows], v[rows]], axis=0).astype(BF16))

            if c < 3:
                put(0, *two_tiles(w, q, c))
                put(1, *two_tiles(w, q, 3 + c))
            else:
                u, v = two_tiles(w, q, 6)
                put(0, jnp.where(lo40, u, 0.0), jnp.where(lo40, v, 0.0))
                put(1, jnp.where(lo40, 0.0, u), jnp.where(lo40, 0.0, v))

        def op_t(q, c):
            project(ar2, ts_s, q, c)

        def op_v(q, c):
            project(ar3, vs_s, q, c)

        slabs = [list(range(5)) if t <= 1 else [0] + list(range(min(t, MINSLAB), 5)) for t in range(5)]
        sc = [None] * 5
        done = []

        def op_s(t, c):
            cols = slice(128 * c, 128 * (c + 1))
            q = jnp.concatenate([h[8 * i:8 * (i + 1), cols] for i in slabs[t]], axis=0)
            if NOXP:
                y = _dot(q, ts_s[t, c])
            else:
                y = _dot(q, ts_s[t, c], NT)
            sc[t] = y if sc[t] is None else sc[t] + y
            done.append((t, c))
            if len(done) == 20:
                softmax_b()

        def op_sb(t):
            for c in range(4):
                op_s(t, c)

        def softmax_b():
            z = [{i: sc[t][8 * n:8 * (n + 1)] for n, i in enumerate(slabs[t])} for t in range(5)]
            rel = _iota((8, 128), 0) - (_iota((8, 128), 1) & 7)
            for t in range(1, 5):
                for i in z[t]:
                    if 1 <= i <= t:
                        z[t][i] = jnp.where(rel >= 8 * (t - i), z[t][i], NEG)
            mx = [functools.reduce(jnp.maximum, [z[t][i] for t in range(5) if i in z[t]]) for i in range(5)]
            mx = _group8_allreduce(jnp.concatenate(mx, axis=0), jnp.maximum)
            for t in range(5):
                for i in z[t]:
                    z[t][i] = jnp.exp2(z[t][i] - mx[8 * i:8 * (i + 1)])
            ls = [functools.reduce(jnp.add, [z[t][i] for t in range(5) if i in z[t]]) for i in range(5)]
            inv = 1.0 / _group8_allreduce(jnp.concatenate(ls, axis=0), jnp.add)
            st["p"] = [jnp.concatenate([z[t][i] * inv[8 * i:8 * (i + 1)] for i in slabs[t]], axis=0)
                       for t in range(5)]

        acc = [[None] * 5 for _ in range(4)]

        def op_p(t, c):
            y = _dot(st["p"][t], vs_s[t, c])
            for n, i in enumerate(slabs[t]):
                yi = y[8 * n:8 * (n + 1)]
                acc[c][i] = yi if acc[c][i] is None else acc[c][i] + yi
            done.append(("p", t, c))
            if all(("p", u, c) in done for u in range(5)):
                o = jnp.concatenate(acc[c], axis=0)
                if c == 3 and not NOROLL:
                    o = o + pltpu.roll(o, 64, 1)
                b_s[slot, pl.ds(_al(hg * 32, 32), 32), 128 * c:128 * (c + 1)] = o[8:40]
                st["mem", c] = o[0:8]

        def op_pb(c):
            for t in range(5):
                op_p(t, c)

        def op_sa(i):
            tri = _iota((32, 128), 0) <= (_iota((32, 128), 1) & 31)
            row = 2 * _iota((56, 128), 0)
            head = (row >= 28).astype(jnp.int32) + (row >= 56).astype(jnp.int32) + (row >= 84).astype(jnp.int32)
            mine = ((head + i) & 3) == (_iota((56, 128), 1) >> 5)
            one = _to_u32(jnp.where(_iota((16, 128), 0) == 15, 1.0, 0.0).astype(BF16))
            qi = jnp.concatenate([jnp.where(mine, ar1[pl.ds(_al(QT + s * 56, 8), 56), :], jnp.uint32(0)), one], axis=0)
            k0 = KA + 1152 * hg + qb * 64 + 16 * i
            cuts = SACUT if i % 2 == 0 else [144 - c for c in SACUT[::-1]]
            sa = jnp.concatenate([_dot(_to_bf16(ar1[pl.ds(_al(k0 + a, 8), b - a), :]), _to_bf16(qi))
                                  for a, b in zip(cuts[:-1], cuts[1:])], axis=0)
            sa = jnp.concatenate([jnp.where(tri, sa[256:288], sa[0:32]), sa[32:256]], axis=0)
            p = jnp.exp2(sa - jnp.max(sa, axis=0, keepdims=True))
            st["l", i] = jnp.broadcast_to(jnp.sum(p, axis=0, keepdims=True), (8, 128))
            p = jnp.concatenate([jnp.where(tri, 0.0, p[0:32]), p[32:256], jnp.where(tri, p[0:32], 0.0)], axis=0)
            pz_s[i] = _to_u32(p.astype(BF16))

        def op_rg(part):
            if part == 0:
                st["inv"] = _regroup([1.0 / st["l", k] for k in range(4)])
            zero = jnp.zeros((16, 128), U32)
            if True:
                for r in range(3 * part, 3 * part + 3):
                    z = [pz_s[k, 16 * (r - k):16 * (r - k + 1), :] if 0 <= r - k <= 8 else zero for k in range(4)]
                    for j, v in enumerate(_regroup(z)):
                        pa_s[j, 16 * r:16 * (r + 1), :] = v

        def op_pa(j):
            w0 = HEAD_WIN[j]
            v = jnp.concatenate([ar1[pl.ds(_al(VT + 2016 * hg + (qb + i) * 112 + w0, 8), 32), :] for i in range(3)], axis=1)
            v = pltpu.bitcast(v, F32)
            o = _dot(v, _to_bf16(pa_s[j])) * jnp.concatenate([st["inv"][j]] * 4, axis=0)
            st["o", j] = pltpu.roll(o, 128 - 32 * j, 1) if j else o
            if all(("o", i) in st for i in range(4)):
                ot = _join_heads([st["o", i] for i in range(4)])
                oa_s[slot, pl.ds(_al(hg * 56, 8), 56), :] = _to_u32(ot.astype(BF16))

        def op_fin():
            finalize(1 - slot, hg, jnp.maximum(qb - 1, 0))

        ops = dict(s=op_s, p=op_p, rg=op_rg, t=op_t, v=op_v, sb=op_sb, pb=op_pb, sa=op_sa, pa=op_pa, fin=op_fin,
                   tr=lambda: transpose_b(1 - slot, hg))
        for name in (LAST if LAST and last else ORDER).split():
            base = name.rstrip("0123456789")
            ops[base](*[int(ch) for ch in name[len(base):]])
        return jnp.concatenate([st["mem", c] for c in range(4)], axis=1)

    def block(qb, mem):
        if not NODMA:
            @pl.when(qb >= 2)
            def _():
                out_copy(qb - 2).start()

        def body(i, mem):
            for u in range(UNROLL):
                mem = step(qb, i * UNROLL + u, mem, u == UNROLL - 1)
            return mem

        if UNROLL == 4:
            return body(0, mem)
        return lax.fori_loop(0, 4 // UNROLL, body, mem)

    m0 = mem0_v[...].astype(F32)
    with _scope('main'):
        lax.fori_loop(0, NQB, block, jnp.concatenate([m0, m0[:, 384:448]], axis=1))

    if NODMA:
        for blk in range(NQB - 2):
            out_copy(blk).start()
    out_copy(NQB - 2).start()
    for hg in range(4):
        transpose_b(1, hg)
        finalize(1, hg, NQB - 1)
    out_copy(NQB - 1).start()
    for blk in range(NQB):
        out_copy(blk).wait()


@functools.partial(jax.jit, static_argnames=("B_seg_len",))
def pallas_gated_mix__sliding_block__memory_aug_recurrent_mem_tr__prompt_kernel(
        A_x, A_wqkv, A_wo, B_x, B_mem0, B_Wq, B_Wk, B_Wv, B_Wo, B_seg_len, gate_w):
    del B_x
    assert A_x.shape == (1, 2048, 448) and B_Wq.shape == (448, 16, 256)
    assert B_mem0.shape == (1, 8, 448) and int(B_seg_len) == 32
    S, D = 2048, 448
    flat = lambda w: w.reshape(D * 16, 256)
    hbm = pl.BlockSpec(memory_space=pltpu.HBM)
    vmem = pltpu.VMEM
    out_t = pl.pallas_call(
        _kernel,
        out_shape=jax.ShapeDtypeStruct((1, D, S), BF16),
        in_specs=[hbm] * 9,
        out_specs=hbm,
        scratch_shapes=[
            vmem((D, S), BF16), vmem((D, 3 * D), BF16), vmem((D, D), BF16), vmem((8, D), BF16),
            vmem((D,), BF16),
            vmem((D * 16, 256), BF16), vmem((D * 16, 256), BF16), vmem((D * 16, 256), BF16),
            vmem((16, D, 256), BF16),
            vmem((30592, 128), U32), vmem((19712, 128), U32), vmem((12544, 128), U32),
            vmem((336, 896), U32), vmem((3 * D, 512), F32), vmem((8, D), U32), vmem((D // 2, D), U32), vmem((S, 512), F32),
            vmem((16, 8, 128), F32),
            vmem((2, D // 2, 128), U32), vmem((2, 128, 512), F32), vmem((512, 128), F32),
            vmem((16, D, 128), BF16),
            vmem((5, 4, 128, 128), BF16), vmem((5, 4, 128, 128), BF16), vmem((4, 192, 128), U32), vmem((4, 144, 128), U32),
            pltpu.SemaphoreType.DMA((8,)), pltpu.SemaphoreType.DMA((28,)), pltpu.SemaphoreType.DMA(()),
        ],
        compiler_params=pltpu.CompilerParams(vmem_limit_bytes=100 * 2**20, disable_bounds_checks=NOBC),
        name="mykern",
    )(A_x.transpose(0, 2, 1), A_wqkv, A_wo, B_mem0, flat(B_Wq), flat(B_Wk), flat(B_Wv),
      B_Wo.transpose(0, 2, 1), gate_w)
    return out_t.transpose(0, 2, 1)
```

```python
import functools
import math

import jax
import jax.numpy as jnp
from jax import lax
from jax.experimental import pallas as pl
from jax.experimental.pallas import tpu as pltpu

F32 = jnp.float32
BF16 = jnp.bfloat16
U32 = jnp.uint32

S, D = 2048, 448
NQB = S // 128
NB = 2
LOG2E = math.log2(math.e)
NEG = -1000000000.0
NN = (((1,), (0,)), ((), ()))
NT = (((1,), (1,)), ((), ()))
HEAD_WIN = (0, 24, 56, 80)

WQ, WK = 0, 7168
KA = 14336
QT = 18944
VT = 22528
WV = 12544

ORDER = (
    "e00 e03 t00 t02 t12 t22 t32 t10 t11 t30 tr t01 t21 t20 t31 v02 sa0 sb1 sb0 v12 sa1 sb2 v22 sa2 sb3 "
    "v32 sa3 sb4 rg0 v00 v10 v30 rg2 v20 rg1 rg3 v01 v11 v21 pb3 v31 pb2 pa1 pa3 pb0 pa2 fin pb1 pa0|")
NOPRO = False


def _dot(a, b, dims=NN):
    return lax.dot_general(a, b, dims, preferred_element_type=F32)


def _to_u32(x_bf16):
    return pltpu.bitcast(x_bf16, U32)


def _to_bf16(x_u32):
    return pltpu.bitcast(x_u32, BF16)


def _iota(shape, dim):
    return lax.broadcasted_iota(jnp.int32, shape, dim)


def _rows(start, size, align):
    return pl.ds(start if isinstance(start, int) else pl.multiple_of(start, align), size)


def _group8_allreduce(x, op):
    lane = _iota(x.shape, 1)
    for d in (1, 2, 4):
        x = op(x, jnp.where((lane & d) == 0, pltpu.roll(x, 128 - d, 1), pltpu.roll(x, d, 1)))
    return x


def _join_heads(w):
    first4 = _iota((8, w[0].shape[1]), 0) < 4
    return jnp.concatenate([
        w[0][0:24], jnp.where(first4, w[0][24:32], w[1][0:8]), w[1][8:32],
        w[2][0:24], jnp.where(first4, w[2][24:32], w[3][0:8]), w[3][8:32]], axis=0)


def _regroup(z):
    lane = _iota(z[0].shape, 1)
    y = [jnp.where((lane & 32) != 0, z[(k + 1) % 4], z[k]) for k in range(4)]
    x = [jnp.where((lane & 64) != 0, y[(k + 2) % 4], y[k]) for k in range(4)]
    return [x[(-j) % 4] for j in range(4)]


def _mixed_chunks(u, v):
    lo = _iota((u.shape[0], 128), 1) < 64
    u2, u3, v2, v3 = u[:, 0:128], u[:, 128:256], v[:, 0:128], v[:, 128:256]
    return jnp.where(lo, u2, u2 - v2), jnp.where(lo, v2, v3 - u3), jnp.where(lo, u3, v2)


def _on_iteration(i, plan):
    for j, actions in enumerate(plan):
        @pl.when(i == j)
        def _():
            for action in actions:
                action()


def _kernel(xt_hbm, wqkv_hbm, wo_hbm, mem0_hbm, wq_hbm, wk_hbm, wv_hbm, bwo_hbm, gw_hbm,
            out_hbm,
            xt_v, wqkv_v, wo_v, mem0_v, gw_v, wq_v, wk_v, wv_v, bwo_v,
            ar1, ar2, ar3, wa_s, wat_s, wof_s, gw_s, wot_s, xn_s, g_s, oa_s, b_s, bt_s, out_v,
            ts_s, vs_s, pa_s, pz_s, sems, osem):
    a_v = pltpu.make_async_copy(wqkv_hbm.at[:, 2 * D:3 * D], wqkv_v.at[:, 2 * D:3 * D], sems.at[0])
    a_qk = pltpu.make_async_copy(wqkv_hbm.at[:, 0:2 * D], wqkv_v.at[:, 0:2 * D], sems.at[1])
    a_o = pltpu.make_async_copy(wo_hbm, wo_v, sems.at[2])
    gate = pltpu.make_async_copy(gw_hbm, gw_v, sems.at[3])
    mem0 = pltpu.make_async_copy(mem0_hbm.at[0], mem0_v, sems.at[4])

    def x_copy(i):
        cols = slice(*(0, 256, 512, 1024, S)[i:i + 2])
        return pltpu.make_async_copy(xt_hbm.at[0, :, cols], xt_v.at[:, cols], sems.at[5 + i])

    def w_copy(which, i):
        src, dst = ((wq_hbm, wq_v), (wk_hbm, wk_v), (wv_hbm, wv_v), (bwo_hbm, bwo_v))[which]
        part = pl.ds(src.shape[0] // 4 * i, src.shape[0] // 4)
        return pltpu.make_async_copy(src.at[part], dst.at[part], sems.at[9 + 4 * which + i])

    start = lambda *copies: [c.start for c in copies]
    wait = lambda *copies: [c.wait for c in copies]

    a_v.start()
    gate.start()
    x_copy(0).start()

    kpad = _to_u32(jnp.where(_iota((128, 128), 1) == 127, NEG, 0.0).astype(BF16))
    for hg in range(4):
        for r in range(0, 128, 64):
            ar1[_rows(KA + 1152 * hg + r, 64, 8), :] = kpad
        for r in range(0, 224, 56):
            ar1[_rows(VT + 2016 * hg + r, 56, 8), :] = jnp.zeros((56, 128), U32)
    for r in range(0, 224, 56):
        oa_s[1, r:r + 56, :] = jnp.zeros((56, 128), U32)
    for r in range(0, 128, 16):
        b_s[1, r:r + 16, :] = jnp.zeros((16, 512), F32)

    def transpose_wqkv(part, chunks):
        for c in chunks:
            n = min(128, 3 * D - c)
            w = wqkv_v[:, c:c + n]
            w = _to_u32(jnp.concatenate([w, w[384:448]], axis=0).T)
            for r in range(0, n, 32):
                half, row = (c + r) % D // 224, (c + r) // D * 224 + (c + r) % 224
                wa_s[row // 2:row // 2 + 16, 384 * half:384 * half + 256] = w[r // 2:r // 2 + 16, 0:256]
                wat_s[(c + r) // 2:(c + r) // 2 + 16, :] = w[r // 2:r // 2 + 16, 256:512]
        for r in range(0, 224, 32):
            u, v = (_to_bf16(wat_s[(D * part + o) // 2:(D * part + o) // 2 + 16, :]).astype(F32)
                    for o in (r, 224 + r))
            dst = slice((224 * part + r) // 2, (224 * part + r) // 2 + 16)
            for col, w in zip((256, 640, 768), _mixed_chunks(u, v)):
                wa_s[dst, col:col + 128] = _to_u32(w.astype(BF16))

    def project_a(qb, part, transpose_x=False, extra=lambda g: None):
        if NOPRO:
            return
        xt = xt_v[:, _rows(qb * 128, 128, 128)]
        x1 = xt[0:384]
        x2 = jnp.concatenate([xt[0:320], xt[384:448]], axis=0)
        x3 = jnp.concatenate([xt[384:448], xt[320:384]], axis=0)
        if part == 0:
            g_s[qb] = jax.nn.sigmoid(_dot(_to_bf16(gw_s[...]), xt)[0:8])
        if transpose_x:
            xn_s[_rows(qb * 128, 128, 128), :] = jnp.concatenate([xt, xt[384:448]], axis=0).T.astype(F32)
        for g in range(2):
            rows = slice(112 * part + 56 * g, 112 * part + 56 * (g + 1))
            shared = _dot(_to_bf16(wa_s[rows, 768:896]), x3)
            for hg, y in ((g, _dot(_to_bf16(wa_s[rows, 0:384]), x1) + shared),
                          (g + 2, _dot(_to_bf16(wa_s[rows, 384:768]), x2) + shared)):
                if part == 0:
                    y = y * (28.0 ** -0.5 * LOG2E)
                    y = _join_heads([y[0:32]] + [pltpu.roll(y[w:w + 32], 32 * j, 1)
                                                 for j, w in enumerate(HEAD_WIN) if j])
                    ar1[_rows(QT + (qb * 4 + hg) * 56, 56, 8), :] = _to_u32(y.astype(BF16))
                elif part == 1:
                    y = jnp.concatenate([y, jnp.zeros((16, 128), F32)], axis=0).astype(BF16)
                    ar1[_rows(KA + 1152 * hg + 128 + qb * 64, 64, 64), :] = _to_u32(y.T)
                else:
                    ar1[_rows(VT + 2016 * hg + (qb + 2) * 112, 112, 16), :] = pltpu.bitcast(y, U32)
            extra(g)

    def deinterleave(src, dst, base, r):
        for c in range(2):
            v = _to_u32(src[_rows(r * 128, 128, 128), c * 128:(c + 1) * 128])
            v = jnp.swapaxes(v.reshape(8, 8, 128), 0, 1)
            for p in range(8):
                dst[_rows(base + (2 * p + c) * D + r * 8, 8, 8), :] = v[p]

    gate.wait()
    a_qk.start()
    a_v.wait()
    x_copy(0).wait()
    gw_s[...] = _to_u32(jnp.broadcast_to(gw_v[...].astype(F32).reshape(1, D), (16, D)).astype(BF16))
    transpose_wqkv(2, range(896, 3 * D, 128))
    project_a(0, 2)
    project_a(1, 2, True)
    a_qk.wait()
    for c in (x_copy(1), x_copy(2), x_copy(3), w_copy(0, 0), w_copy(1, 0)):
        c.start()
    transpose_wqkv(1, range(384, 896, 128))
    project_a(0, 1)
    transpose_wqkv(0, range(0, 384, 128))
    project_a(1, 1)
    project_a(0, 0, True)
    project_a(1, 0)

    def project_early(i, carry):
        _on_iteration(i, [wait(x_copy(1)) + start(w_copy(0, 1), w_copy(1, 1)),
                          wait(x_copy(2)) + start(w_copy(0, 2), w_copy(1, 2)),
                          start(w_copy(0, 3), w_copy(1, 3))])
        for u in range(2):
            for part in (1, 0, 2):
                project_a(2 * i + 2 + u, part, part == 1)
        return carry

    lax.fori_loop(0, 3, project_early, 0)

    def project_late(i, carry):
        _on_iteration(i, [wait(x_copy(3), w_copy(0, 0), w_copy(1, 0)),
                          wait(w_copy(0, 1), w_copy(1, 1)) + start(w_copy(2, 0), w_copy(2, 1)),
                          wait(w_copy(0, 2), w_copy(1, 2)) + start(w_copy(2, 2), w_copy(2, 3)),
                          wait(w_copy(0, 3), w_copy(1, 3)) + start(a_o, mem0)])
        cuts = (0, 3, 5, 7, 10, 12, 14)
        for u in range(2):
            for m, part in enumerate((1, 0, 2)):
                def extra(g):
                    for j in range(cuts[2 * m + g], cuts[2 * m + g + 1]):
                        src, base = (wq_v, WQ) if j < 7 else (wk_v, WK)
                        deinterleave(src, ar1, base, (2 * i + u) * 7 + j % 7)

                project_a(2 * i + 8 + u, part, part == 1, extra)
        return carry

    lax.fori_loop(0, 4, project_late, 0)

    def head_rows(src, base, q, k, r0=0, n=D):
        p = 2 * q + k // 2
        w = jnp.concatenate([src[_rows(base + (2 * p + c) * D + r0, n, 64), :] for c in range(2)], axis=1)
        return pltpu.bitcast(w << 16 if k % 2 == 0 else w & jnp.uint32(0xFFFF0000), F32)

    def merge(dst, q, lhs, rhs, extra=lambda k: None):
        if NOPRO:
            return

        def put(tile, u, v):
            u3 = u[384:448].astype(BF16)
            v2 = v[320:384].astype(BF16)
            dst[_rows((q * 7 + tile) * D, D, 64), :] = _to_u32(jnp.concatenate([
                u[0:320].astype(BF16), (u[320:384] - v2.astype(F32)).astype(BF16),
                v[0:320].astype(BF16), (v[384:448] - u3.astype(F32)).astype(BF16),
                u3, v2], axis=0))

        def block(i, c):
            put(3 * i + c, _dot(lhs(i), rhs(i, 128 * c, 128), NT), _dot(lhs(2 + i), rhs(2 + i, 128 * c, 128), NT))

        block(0, 0)
        extra(0)
        tail = [jnp.concatenate([_dot(rhs(k, 384, 64), lhs(k).astype(BF16), NT) for k in (i, i + 1)], axis=0)
                for i in (0, 2)]
        block(0, 1)
        extra(1)
        block(0, 2)
        extra(2)
        put(6, tail[0].T, tail[1].T)
        block(1, 0)
        extra(3)
        block(1, 1)
        extra(4)
        block(1, 2)

    def merge_qk(q, carry):
        _on_iteration(q, [wait(w_copy(2, j)) + start(w_copy(3, j)) for j in range(4)])

        def extra(k):
            for j in range(3 * k, min(3 * k + 3, 14)):
                deinterleave(wv_v, ar2, WV, 14 * q + j)

        merge(ar2, q, functools.partial(head_rows, ar1, WK, q),
              lambda k, r0, n: head_rows(ar1, WQ, q, k, r0, n).astype(BF16), extra)
        return carry

    lax.fori_loop(0, 4, merge_qk, 0)
    a_o.wait()

    def merge_vo(q, carry):
        _on_iteration(q, [wait(w_copy(3, j)) for j in range(4)])
        w = jnp.concatenate([wo_v[_rows(jnp.minimum(128 * q + r, 384), 64, 64), :] for r in (0, 64)], axis=0)
        wof_s[:, _rows(128 * q, 128, 128)] = w.astype(F32).T
        merge(ar3, q, functools.partial(head_rows, ar2, WV, q),
              lambda k, r0, n: bwo_v[4 * q + k, r0:r0 + n, :])
        return carry

    lax.fori_loop(0, 4, merge_vo, 0)
    for k in range(4):
        for r in range(0, 56, 8):
            u, v = (wof_s[112 * k + o:112 * k + o + 8, :] for o in (r, r + 56))
            m = _mixed_chunks(u[:, 256:512], v[:, 256:512])
            wot_s[56 * k + r:56 * k + r + 8, :] = jnp.concatenate(
                [u[:, 0:256], m[0], v[:, 0:256], m[1], m[2]], axis=1)
    mem0.wait()

    def transpose_b(slot, c):
        bt_s[128 * c:128 * (c + 1), :] = b_s[slot, :, 128 * c:128 * (c + 1)].T

    def finalize(slot, k, blk):
        rows = slice(56 * k, 56 * (k + 1))
        o = lambda *cuts: _to_bf16(jnp.concatenate([oa_s[slot, a // 2:b // 2, :] for a, b in cuts], axis=0))
        shared = _dot(wot_s[rows, 768:896], o((384, 448), (320, 384)))
        a = jnp.concatenate([_dot(wot_s[rows, 0:384], o((0, 384))) + shared,
                             _dot(wot_s[rows, 384:768], o((0, 320), (384, 448))) + shared], axis=0)
        g = jnp.broadcast_to(g_s[blk][0:1], (112, 128))
        rows = slice(112 * k, 112 * (k + 1))
        out_v[blk, rows, :] = (g * a + (1.0 - g) * bt_s[rows, :]).astype(BF16)

    def out_copy(blk):
        return pltpu.make_async_copy(out_v.at[blk], out_hbm.at[0, :, _rows(blk * 128, 128, 128)], osem)

    slabs = [list(range(5)) if t <= 1 else [0] + list(range(t, 5)) for t in range(5)]
    tiles = [(t, c) for t in range(5) for c in range(4) if c < 3 or t in (0, 1, 3)]
    slab = lambda y, i: y[8 * i:8 * (i + 1)]
    split = lambda y, t: {i: slab(y, n) for n, i in enumerate(slabs[t])}

    def accumulate(acc, y):
        for i, v in y.items():
            acc[i] = acc[i] + v if i in acc else v

    def step(qb, slot, hg, mem, order):
        s = qb * 4 + hg
        h = jnp.concatenate([mem, xn_s[_rows(s * 32, 32, 32), :]], axis=0)
        lo8 = _iota((8, 128), 1) < 64
        lo40 = _iota((40, 128), 1) < 64
        a12 = h[:, 256:384]
        a13 = jnp.where(lo40, a12, h[:, 384:512])
        a32 = jnp.where(lo40, h[:, 384:512], a12)
        early, scores, probs, outs, done = {}, [{} for _ in range(5)], [], [{} for _ in range(4)], set()
        new_mem, denom, heads = {}, {}, {}

        def early_passes(q, c):
            o = (q * 7 + c) * D
            w = lambda k: _to_bf16(ar2[o + 64 * k:o + 64 * (k + 1), :])
            shared = _dot(a32, w(6))
            early[q, c] = (_dot(h[:, 0:128], w(0)) + _dot(a12, w(2)) + shared,
                           _dot(h[:, 0:128], w(3)) + _dot(a13, w(5)) + shared)

        def two_tiles(w, q, c):
            o = (q * 7 + c) * D
            if w is ar2 and (q, c) in early:
                return (early[q, c][0] + _dot(h[:, 128:256], _to_bf16(w[o + 64:o + 128, :])),
                        early[q, c][1] + _dot(h[:, 128:256], _to_bf16(w[o + 256:o + 320, :])))
            shared = _dot(a32, _to_bf16(w[o + 384:o + 448, :]))
            return (_dot(h[:, 0:384], _to_bf16(w[o:o + 192, :])) + shared,
                    _dot(jnp.concatenate([h[:, 0:256], a13], axis=1), _to_bf16(w[o + 192:o + 384, :])) + shared)

        def project(w, dst, q, c):
            def put(t, c, i, uv):
                dst[t, c, 32 * q + 16 * i:32 * q + 16 * (i + 1), :] = jnp.concatenate(uv, axis=0).astype(BF16)

            if c < 2:
                for i in range(2):
                    y = two_tiles(w, q, 3 * i + c)
                    for t in range(5):
                        put(t, c, i, [slab(v, t) for v in y])
                return
            z = two_tiles(w, q, 6)
            put(0, 3, 0, [jnp.where(lo8, slab(v, 0), 0.0) for v in z])
            put(0, 3, 1, [jnp.where(lo8, 0.0, slab(v, 0)) for v in z])
            dz = {t: [slab(v, t + 1) - slab(v, t) for v in z] for t in (1, 3)}
            moved = {t: [pltpu.roll(jnp.where(lo8, d, slab(v, t)), 64, 1) for d, v in zip(dz[t], z)]
                     for t in (1, 3)}
            for i in range(2):
                y = two_tiles(w, q, 3 * i + 2)
                put(0, 2, i, [slab(v, 0) for v in y])
                for t in (1, 3):
                    hi = moved[t] if i == 0 else dz[t]
                    lo = [slab(v, t) for v in z] if i == 0 else moved[t]
                    put(t, 2, i, [jnp.where(lo8, slab(v, t), slab(v, t) - slab(v, t + 1)) for v in y])
                    put(t + 1, 2, i, [jnp.where(lo8, slab(v, t + 1), e) for v, e in zip(y, hi)])
                    put(t, 3, i, [jnp.where(lo8, e, slab(v, t + 1)) for v, e in zip(y, lo)])

        def scores_b(k):
            for t, c in tiles[4 * k:4 * k + 4]:
                lhs = h[:, 128 * c:128 * (c + 1)] if c < 2 or t == 0 else a32 if c == 3 else a12 if t % 2 else a13
                y = split(_dot(jnp.concatenate([slab(lhs, i) for i in slabs[t]], axis=0), ts_s[t, c], NT), t)
                accumulate(scores[t], y)
                if c == 3 and t:
                    accumulate(scores[t + 1], {i: y[i] for i in slabs[t + 1]})
            done.add(k)
            if len(done) < 5:
                return
            z = [{i: v * (256.0 ** -0.5 * LOG2E) for i, v in sc.items()} for sc in scores]
            causal = _iota((8, 128), 0) >= (_iota((8, 128), 1) & 7)
            for t in range(1, 5):
                z[t][t] = jnp.where(causal, z[t][t], NEG)
            over_keys = lambda op: _group8_allreduce(jnp.concatenate(
                [functools.reduce(op, [zt[i] for zt in z if i in zt]) for i in range(5)], axis=0), op)
            top = over_keys(jnp.maximum)
            z = [{i: jnp.exp2(v - slab(top, i)) for i, v in zt.items()} for zt in z]
            inv = 1.0 / over_keys(jnp.add)
            probs.extend({i: v * slab(inv, i) for i, v in zt.items()} for zt in z)

        def output_b(k):
            todo = ([(t, k) for t in range(5)] if k < 2 else
                    [(0, 2), (1, 2), (3, 2)] if k == 2 else [(0, 3), (1, 3), (2, 2), (3, 3), (4, 2)])
            for t, c in todo:
                p = probs[t]
                if c == 3 and t:
                    p = {i: v + probs[t + 1][i] if i in probs[t + 1] else v for i, v in p.items()}
                y = split(_dot(jnp.concatenate([p[i] for i in slabs[t]], axis=0), vs_s[t, c]), t)
                if c < 2 or t == 0 or (c == 2 and t % 2):
                    accumulate(outs[c], y)
                else:
                    accumulate(outs[5 - c], {i: jnp.where(lo8, 0.0, v) for i, v in y.items()})
                    accumulate(outs[c], {i: jnp.where(lo8, v, 0.0) for i, v in y.items()})
            done.add(("out", k))
            for c in ((k,) if k < 2 else (2, 3) if {("out", 2), ("out", 3)} <= done else ()):
                o = jnp.concatenate([outs[c][i] for i in range(5)], axis=0)
                if c == 3:
                    o = o + pltpu.roll(o, 64, 1)
                b_s[slot, 32 * hg:32 * (hg + 1), 128 * c:128 * (c + 1)] = o[8:40]
                new_mem[c] = o[0:8]

        def softmax_a(i):
            row = 2 * _iota((56, 128), 0)
            head = sum((row >= 28 * j).astype(jnp.int32) for j in (1, 2, 3))
            mine = ((head + i) & 3) == (_iota((56, 128), 1) >> 5)
            ones = _to_u32(jnp.where(_iota((16, 128), 0) == 15, 1.0, 0.0).astype(BF16))
            q = jnp.concatenate([jnp.where(mine, ar1[_rows(QT + s * 56, 56, 8), :], jnp.uint32(0)), ones], axis=0)
            k0 = KA + 1152 * hg + qb * 64 + 16 * i
            cuts = (0, 40, 72, 112, 144) if i % 2 == 0 else (0, 32, 72, 104, 144)
            z = jnp.concatenate([_dot(_to_bf16(ar1[_rows(k0 + a, b - a, 8), :]), _to_bf16(q))
                                 for a, b in zip(cuts[:-1], cuts[1:])], axis=0)
            newest = _iota((32, 128), 0) <= (_iota((32, 128), 1) & 31)
            z = jnp.concatenate([jnp.where(newest, z[256:288], z[0:32]), z[32:256]], axis=0)
            p = jnp.exp2(z - jnp.max(z, axis=0, keepdims=True))
            denom[i] = jnp.broadcast_to(jnp.sum(p, axis=0, keepdims=True), (8, 128))
            pz_s[i] = _to_u32(jnp.concatenate([
                jnp.where(newest, 0.0, p[0:32]), p[32:256], jnp.where(newest, p[0:32], 0.0)], axis=0).astype(BF16))

        def regroup_a(part):
            if part == 0:
                denom["inv"] = _regroup([1.0 / denom[i] for i in range(4)])
            for r in range(3 * part, 3 * part + 3):
                z = [pz_s[i, 16 * (r - i):16 * (r - i + 1), :] if 0 <= r - i <= 8 else jnp.zeros((16, 128), U32)
                     for i in range(4)]
                for j, v in enumerate(_regroup(z)):
                    pa_s[j, 16 * r:16 * (r + 1), :] = v

        def output_a(j):
            v = jnp.concatenate([ar1[_rows(VT + 2016 * hg + (qb + i) * 112 + HEAD_WIN[j], 32, 8), :]
                                 for i in range(3)], axis=1)
            o = _dot(pltpu.bitcast(v, F32), _to_bf16(pa_s[j])) * jnp.concatenate([denom["inv"][j]] * 4, axis=0)
            heads[j] = pltpu.roll(o, 128 - 32 * j, 1) if j else o
            if len(heads) == 4:
                oa_s[slot, 56 * hg:56 * (hg + 1), :] = _to_u32(
                    _join_heads([heads[i] for i in range(4)]).astype(BF16))

        pieces = dict(
            e=early_passes, t=functools.partial(project, ar2, ts_s), v=functools.partial(project, ar3, vs_s),
            sb=scores_b, pb=output_b, sa=softmax_a, rg=regroup_a, pa=output_a,
            tr=lambda: transpose_b(1 - slot, hg),
            fin=lambda: finalize(1 - slot, hg, jnp.maximum(qb - 1, 0)))
        for name in order.split():
            kind = name.rstrip("0123456789")
            pieces[kind](*map(int, name[len(kind):]))
        return jnp.concatenate([new_mem[c] for c in range(4)], axis=1)

    def blocks(i, mem):
        for u in range(NB):
            @pl.when(i * NB + u - NB - 1 >= 0)
            def _():
                out_copy(i * NB + u - NB - 1).start()

        orders = [o for o in ORDER.split("|") if o]
        for u in range(NB):
            for hg in range(4):
                mem = step(i * NB + u, u % 2, hg, mem, orders[(4 * u + hg) % len(orders)])
        return mem

    m0 = mem0_v[...].astype(F32)
    lax.fori_loop(0, NQB // NB, blocks, jnp.concatenate([m0, m0[:, 384:448]], axis=1))

    for blk in range(NQB - NB - 1, NQB - 1):
        out_copy(blk).start()
    for k in range(4):
        transpose_b(1, k)
    for k in range(4):
        finalize(1, k, NQB - 1)
    out_copy(NQB - 1).start()
    for blk in range(NQB):
        out_copy(blk).wait()


@functools.partial(jax.jit, static_argnames=("B_seg_len",))
def pallas_gated_mix__sliding_block__memory_aug_recurrent_mem_tr__prompt_kernel(
        A_x, A_wqkv, A_wo, B_x, B_mem0, B_Wq, B_Wk, B_Wv, B_Wo, B_seg_len, gate_w):
    del B_x
    assert A_x.shape == (1, S, D) and B_Wq.shape == (D, 16, 256)
    assert B_mem0.shape == (1, 8, D) and B_seg_len == 32
    flat = lambda w: w.reshape(D * 16, 256)
    hbm = pl.BlockSpec(memory_space=pltpu.HBM)
    vmem = pltpu.VMEM
    out_t = pl.pallas_call(
        _kernel,
        out_shape=jax.ShapeDtypeStruct((1, D, S), BF16),
        in_specs=[hbm] * 9,
        out_specs=hbm,
        scratch_shapes=[
            vmem((D, S), BF16), vmem((D, 3 * D), BF16), vmem((D, D), BF16), vmem((8, D), BF16), vmem((D,), BF16),
            vmem((D * 16, 256), BF16), vmem((D * 16, 256), BF16), vmem((D * 16, 256), BF16),
            vmem((16, D, 256), BF16),
            vmem((30592, 128), U32), vmem((19712, 128), U32), vmem((12544, 128), U32),
            vmem((336, 896), U32), vmem((672, 256), U32), vmem((D, 512), F32), vmem((8, D), U32),
            vmem((224, 896), F32), vmem((S, 512), F32), vmem((NQB, 8, 128), F32),
            vmem((2, 224, 128), U32), vmem((2, 128, 512), F32), vmem((512, 128), F32), vmem((NQB, D, 128), BF16),
            vmem((5, 4, 128, 128), BF16), vmem((5, 4, 128, 128), BF16),
            vmem((4, 192, 128), U32), vmem((4, 144, 128), U32),
            pltpu.SemaphoreType.DMA((25,)), pltpu.SemaphoreType.DMA(()),
        ],
        compiler_params=pltpu.CompilerParams(vmem_limit_bytes=100 * 2**20),
        name="mykern",
    )(A_x.transpose(0, 2, 1), A_wqkv, A_wo, B_mem0, flat(B_Wq), flat(B_Wk), flat(B_Wv),
      B_Wo.transpose(0, 2, 1), gate_w)
    return out_t.transpose(0, 2, 1)
```

```python
import functools
import math

import jax
import jax.numpy as jnp
from jax import lax
from jax.experimental import pallas as pl
from jax.experimental.pallas import tpu as pltpu

F32 = jnp.float32
BF16 = jnp.bfloat16
U32 = jnp.uint32

S, D = 2048, 448
NQB = S // 128
NB = 2
LOG2E = math.log2(math.e)
NEG = -1000000000.0
NN = (((1,), (0,)), ((), ()))
NT = (((1,), (1,)), ((), ()))
HEAD_WIN = (0, 24, 56, 80)

WQ, WK = 0, 7168
KA = 14336
QT = 18944
VT = 22528
WV = 12544

ORDER = (
    "e00 e03 t12 t02 t22 t32 t00 t10 t31 t30 t20 tr t21 t01 t11 v02 sa0 sb0 sb1 v12 sb2 sa1 v22 sb3 sa2 v32 "
    "sa3 rg0 sb4 v30 v20 v10 v21 v00 rg2 rg1 rg3 v31 v11 pb3 v01 pb2 pa3 pa1 pb0 pa2 fin pb1 pa0|"
    "e03 e00 t00 t12 t02 t22 t10 t31 t30 t32 t21 t11 t20 tr t01 v02 sa0 sb0 sb1 v12 sb2 sa1 v22 sa2 sb3 v32 "
    "sa3 sb4 v30 rg0 v20 v10 rg2 rg1 v00 rg3 v31 v21 v11 pb3 v01 pb2 pa1 pa3 pb0 pa2 fin pb1 pa0|"
    "e00 e03 t00 t12 t02 t22 t32 t10 t31 t30 t20 t21 tr t11 t01 v02 sa0 sb1 sb0 v12 sa1 sb2 v22 sb3 sa2 v32 "
    "sa3 sb4 rg0 v30 v20 v10 v21 v31 rg2 v00 rg1 rg3 v11 pb3 v01 pb2 pa3 pa1 pb0 pa2 fin pb1 pa0|"
    "e00 e03 t00 t12 t02 t22 t32 t10 t31 t30 t20 t21 tr t11 t01 v02 sa0 sb1 sb0 v12 sa1 sb2 v22 sb3 sa2 v32 "
    "sa3 sb4 rg0 v30 v20 v10 v21 v31 rg2 v00 rg1 rg3 v11 pb3 v01 pb2 pa1 pa3 pb0 pa2 fin pb1 pa0|"
    "e03 e00 t00 t12 t02 t22 t32 t10 t31 t30 t21 t11 t20 t01 v02 sb1 sa0 sb0 v12 tr sa1 sb2 v22 sa2 sb3 v32 "
    "sa3 rg0 sb4 v30 v20 rg1 v10 v00 rg3 v11 v31 rg2 v21 pb3 v01 pb2 pa1 pa3 pb0 pa2 fin pb1 pa0|"
    "e00 e03 t00 t12 t02 t22 t32 t10 t31 t30 tr t21 t11 t20 t01 v02 sb1 sa0 sb0 v12 sb2 sa1 sb3 v22 sa2 v32 "
    "sa3 sb4 v30 v20 rg0 v10 rg2 v00 rg3 v31 rg1 v21 v11 pb3 v01 pb2 pa1 pa3 pb0 pa2 fin pb1 pa0|"
    "e03 e00 t00 t02 t12 t22 t32 t30 t21 t10 t31 tr t11 t20 t01 v02 sa0 sb1 sb0 v12 sa1 sb2 v22 sa2 sb3 v32 "
    "sa3 sb4 v30 v20 v10 rg0 v00 rg1 rg3 v31 v21 v11 rg2 pb3 v01 pb2 pa1 pa3 pb0 pa2 fin pb1 pa0|"
    "e00 e03 t00 t12 t02 t22 t32 t10 t30 t31 tr t21 t11 t20 t01 v02 sa0 sb1 sb0 v12 sa1 sb2 v22 sa2 sb3 v32 "
    "sa3 sb4 rg0 v30 rg1 v20 v10 rg2 v00 rg3 v31 v21 pa3 pa1 v11 pa0 pa2 pb3 v01 pb2 fin pb0 pb1|")


def _dot(a, b, dims=NN):
    return lax.dot_general(a, b, dims, preferred_element_type=F32)


def _to_u32(x_bf16):
    return pltpu.bitcast(x_bf16, U32)


def _to_bf16(x_u32):
    return pltpu.bitcast(x_u32, BF16)


def _iota(shape, dim):
    return lax.broadcasted_iota(jnp.int32, shape, dim)


def _rows(start, size, align):
    return pl.ds(start if isinstance(start, int) else pl.multiple_of(start, align), size)


def _group8_allreduce(x, op):
    lane = _iota(x.shape, 1)
    for d in (1, 2, 4):
        x = op(x, jnp.where((lane & d) == 0, pltpu.roll(x, 128 - d, 1), pltpu.roll(x, d, 1)))
    return x


def _join_heads(w):
    first4 = _iota((8, w[0].shape[1]), 0) < 4
    return jnp.concatenate([
        w[0][0:24], jnp.where(first4, w[0][24:32], w[1][0:8]), w[1][8:32],
        w[2][0:24], jnp.where(first4, w[2][24:32], w[3][0:8]), w[3][8:32]], axis=0)


def _regroup(z):
    lane = _iota(z[0].shape, 1)
    y = [jnp.where((lane & 32) != 0, z[(k + 1) % 4], z[k]) for k in range(4)]
    x = [jnp.where((lane & 64) != 0, y[(k + 2) % 4], y[k]) for k in range(4)]
    return [x[(-j) % 4] for j in range(4)]


def _mixed_chunks(u, v):
    lo = _iota((u.shape[0], 128), 1) < 64
    u2, u3, v2, v3 = u[:, 0:128], u[:, 128:256], v[:, 0:128], v[:, 128:256]
    return jnp.where(lo, u2, u2 - v2), jnp.where(lo, v2, v3 - u3), jnp.where(lo, u3, v2)


def _on_iteration(i, plan):
    for j, actions in enumerate(plan):
        @pl.when(i == j)
        def _():
            for action in actions:
                action()


def _kernel(xt_hbm, wqkv_hbm, wo_hbm, mem0_hbm, wq_hbm, wk_hbm, wv_hbm, bwo_hbm, gw_hbm,
            out_hbm,
            xt_v, wqkv_v, wo_v, mem0_v, gw_v, wq_v, wk_v, wv_v, bwo_v,
            ar1, ar2, ar3, wa_s, wat_s, wof_s, gw_s, wot_s, xn_s, g_s, oa_s, b_s, bt_s, out_v,
            ts_s, vs_s, pa_s, pz_s, sems, osem):
    a_v = pltpu.make_async_copy(wqkv_hbm.at[:, 2 * D:3 * D], wqkv_v.at[:, 2 * D:3 * D], sems.at[0])
    a_qk = pltpu.make_async_copy(wqkv_hbm.at[:, 0:2 * D], wqkv_v.at[:, 0:2 * D], sems.at[1])
    a_o = pltpu.make_async_copy(wo_hbm, wo_v, sems.at[2])
    gate = pltpu.make_async_copy(gw_hbm, gw_v, sems.at[3])
    mem0 = pltpu.make_async_copy(mem0_hbm.at[0], mem0_v, sems.at[4])

    def x_copy(i):
        cols = slice(*(0, 256, 512, 1024, S)[i:i + 2])
        return pltpu.make_async_copy(xt_hbm.at[0, :, cols], xt_v.at[:, cols], sems.at[5 + i])

    def w_copy(which, i):
        src, dst = ((wq_hbm, wq_v), (wk_hbm, wk_v), (wv_hbm, wv_v), (bwo_hbm, bwo_v))[which]
        part = pl.ds(src.shape[0] // 4 * i, src.shape[0] // 4)
        return pltpu.make_async_copy(src.at[part], dst.at[part], sems.at[9 + 4 * which + i])

    start = lambda *copies: [c.start for c in copies]
    wait = lambda *copies: [c.wait for c in copies]

    a_v.start()
    gate.start()
    x_copy(0).start()

    kpad = _to_u32(jnp.where(_iota((128, 128), 1) == 127, NEG, 0.0).astype(BF16))
    for hg in range(4):
        for r in range(0, 128, 64):
            ar1[_rows(KA + 1152 * hg + r, 64, 8), :] = kpad
        for r in range(0, 224, 56):
            ar1[_rows(VT + 2016 * hg + r, 56, 8), :] = jnp.zeros((56, 128), U32)
    for r in range(0, 224, 56):
        oa_s[1, r:r + 56, :] = jnp.zeros((56, 128), U32)
    for r in range(0, 128, 16):
        b_s[1, r:r + 16, :] = jnp.zeros((16, 512), F32)

    def transpose_wqkv(part, chunks):
        for c in chunks:
            n = min(128, 3 * D - c)
            w = wqkv_v[:, c:c + n]
            w = _to_u32(jnp.concatenate([w, w[384:448]], axis=0).T)
            for r in range(0, n, 32):
                half, row = (c + r) % D // 224, (c + r) // D * 224 + (c + r) % 224
                wa_s[row // 2:row // 2 + 16, 384 * half:384 * half + 256] = w[r // 2:r // 2 + 16, 0:256]
                wat_s[(c + r) // 2:(c + r) // 2 + 16, :] = w[r // 2:r // 2 + 16, 256:512]
        for r in range(0, 224, 32):
            u, v = (_to_bf16(wat_s[(D * part + o) // 2:(D * part + o) // 2 + 16, :]).astype(F32)
                    for o in (r, 224 + r))
            dst = slice((224 * part + r) // 2, (224 * part + r) // 2 + 16)
            for col, w in zip((256, 640, 768), _mixed_chunks(u, v)):
                wa_s[dst, col:col + 128] = _to_u32(w.astype(BF16))

    def project_a(qb, part, transpose_x=False, extra=lambda g: None):
        xt = xt_v[:, _rows(qb * 128, 128, 128)]
        x1 = xt[0:384]
        x2 = jnp.concatenate([xt[0:320], xt[384:448]], axis=0)
        x3 = jnp.concatenate([xt[384:448], xt[320:384]], axis=0)
        if part == 0:
            g_s[qb] = jax.nn.sigmoid(_dot(gw_s[...], xt))
        if transpose_x:
            xn_s[_rows(qb * 128, 128, 128), :] = jnp.concatenate([xt, xt[384:448]], axis=0).T.astype(F32)
        for g in range(2):
            rows = slice(112 * part + 56 * g, 112 * part + 56 * (g + 1))
            shared = _dot(_to_bf16(wa_s[rows, 768:896]), x3)
            for hg, y in ((g, _dot(_to_bf16(wa_s[rows, 0:384]), x1) + shared),
                          (g + 2, _dot(_to_bf16(wa_s[rows, 384:768]), x2) + shared)):
                if part == 0:
                    y = y * (28.0 ** -0.5 * LOG2E)
                    y = _join_heads([y[0:32]] + [pltpu.roll(y[w:w + 32], 32 * j, 1)
                                                 for j, w in enumerate(HEAD_WIN) if j])
                    ar1[_rows(QT + (qb * 4 + hg) * 56, 56, 8), :] = _to_u32(y.astype(BF16))
                elif part == 1:
                    y = jnp.concatenate([y, jnp.zeros((16, 128), F32)], axis=0).astype(BF16)
                    ar1[_rows(KA + 1152 * hg + 128 + qb * 64, 64, 64), :] = _to_u32(y.T)
                else:
                    ar1[_rows(VT + 2016 * hg + (qb + 2) * 112, 112, 16), :] = pltpu.bitcast(y, U32)
            extra(g)

    def deinterleave(src, dst, base, r):
        for c in range(2):
            v = _to_u32(src[_rows(r * 128, 128, 128), c * 128:(c + 1) * 128])
            v = jnp.swapaxes(v.reshape(8, 8, 128), 0, 1)
            for p in range(8):
                dst[_rows(base + (2 * p + c) * D + r * 8, 8, 8), :] = v[p]

    gate.wait()
    a_qk.start()
    a_v.wait()
    x_copy(0).wait()
    gw_s[...] = jnp.broadcast_to(gw_v[...].astype(F32).reshape(1, D), (8, D))
    transpose_wqkv(2, range(896, 3 * D, 128))
    project_a(0, 2)
    project_a(1, 2, True)
    a_qk.wait()
    for c in (x_copy(1), x_copy(2), x_copy(3), w_copy(0, 0), w_copy(1, 0)):
        c.start()
    transpose_wqkv(1, range(384, 896, 128))
    project_a(0, 1)
    transpose_wqkv(0, range(0, 384, 128))
    project_a(1, 1)
    project_a(0, 0, True)
    project_a(1, 0)

    def project_early(i, carry):
        _on_iteration(i, [wait(x_copy(1)) + start(w_copy(0, 1), w_copy(1, 1)),
                          wait(x_copy(2)) + start(w_copy(0, 2), w_copy(1, 2)),
                          start(w_copy(0, 3), w_copy(1, 3))])
        for u in range(2):
            for part in (1, 0, 2):
                project_a(2 * i + 2 + u, part, part == 1)
        return carry

    lax.fori_loop(0, 3, project_early, 0)

    def project_late(i, carry):
        _on_iteration(i, [wait(x_copy(3), w_copy(0, 0), w_copy(1, 0)),
                          wait(w_copy(0, 1), w_copy(1, 1)) + start(w_copy(2, 0), w_copy(2, 1)),
                          wait(w_copy(0, 2), w_copy(1, 2)) + start(w_copy(2, 2), w_copy(2, 3)),
                          wait(w_copy(0, 3), w_copy(1, 3)) + start(a_o, mem0)])
        cuts = (0, 3, 5, 7, 10, 12, 14)
        for u in range(2):
            for m, part in enumerate((1, 0, 2)):
                def extra(g):
                    for j in range(cuts[2 * m + g], cuts[2 * m + g + 1]):
                        src, base = (wq_v, WQ) if j < 7 else (wk_v, WK)
                        deinterleave(src, ar1, base, (2 * i + u) * 7 + j % 7)

                project_a(2 * i + 8 + u, part, part == 1, extra)
        return carry

    lax.fori_loop(0, 4, project_late, 0)

    def head_rows(src, base, q, k, r0=0, n=D):
        p = 2 * q + k // 2
        w = jnp.concatenate([src[_rows(base + (2 * p + c) * D + r0, n, 64), :] for c in range(2)], axis=1)
        return pltpu.bitcast(w << 16 if k % 2 == 0 else w & jnp.uint32(0xFFFF0000), F32)

    def merge(dst, q, lhs, rhs, extra=lambda k: None):
        def put(tile, u, v):
            u3 = u[384:448].astype(BF16)
            v2 = v[320:384].astype(BF16)
            dst[_rows((q * 7 + tile) * D, D, 64), :] = _to_u32(jnp.concatenate([
                u[0:320].astype(BF16), (u[320:384] - v2.astype(F32)).astype(BF16),
                v[0:320].astype(BF16), (v[384:448] - u3.astype(F32)).astype(BF16),
                u3, v2], axis=0))

        def block(i, c):
            put(3 * i + c, _dot(lhs(i), rhs(i, 128 * c, 128), NT), _dot(lhs(2 + i), rhs(2 + i, 128 * c, 128), NT))

        block(0, 0)
        extra(0)
        tail = [jnp.concatenate([_dot(rhs(k, 384, 64), lhs(k).astype(BF16), NT) for k in (i, i + 1)], axis=0)
                for i in (0, 2)]
        block(0, 1)
        extra(1)
        block(0, 2)
        extra(2)
        put(6, tail[0].T, tail[1].T)
        block(1, 0)
        extra(3)
        block(1, 1)
        extra(4)
        block(1, 2)

    def merge_qk(q, carry):
        _on_iteration(q, [wait(w_copy(2, 0)) + start(w_copy(3, 0), w_copy(3, 1)),
                          wait(w_copy(2, 1)) + start(w_copy(3, 2), w_copy(3, 3)),
                          wait(w_copy(2, 2)), wait(w_copy(2, 3))])

        def extra(k):
            for j in range(3 * k, min(3 * k + 3, 14)):
                deinterleave(wv_v, ar2, WV, 14 * q + j)

        merge(ar2, q, functools.partial(head_rows, ar1, WK, q),
              lambda k, r0, n: head_rows(ar1, WQ, q, k, r0, n).astype(BF16), extra)
        return carry

    lax.fori_loop(0, 4, merge_qk, 0)
    for c in [a_o] + [w_copy(3, q) for q in range(4)]:
        c.wait()
    for q in range(4):
        w = jnp.concatenate([wo_v[_rows(min(128 * q + r, 384), 64, 64), :] for r in (0, 64)], axis=0)
        wof_s[:, 128 * q:128 * (q + 1)] = w.astype(F32).T
        merge(ar3, q, functools.partial(head_rows, ar2, WV, q),
              lambda k, r0, n: bwo_v[4 * q + k, r0:r0 + n, :])
    for k in range(4):
        for r in range(0, 56, 8):
            u, v = (wof_s[112 * k + o:112 * k + o + 8, :] for o in (r, r + 56))
            m = _mixed_chunks(u[:, 256:512], v[:, 256:512])
            wot_s[56 * k + r:56 * k + r + 8, :] = jnp.concatenate(
                [u[:, 0:256], m[0], v[:, 0:256], m[1], m[2]], axis=1)
    mem0.wait()

    def transpose_b(slot, c):
        bt_s[128 * c:128 * (c + 1), :] = b_s[slot, :, 128 * c:128 * (c + 1)].T

    def finalize(slot, k, blk):
        rows = slice(56 * k, 56 * (k + 1))
        o = lambda *cuts: _to_bf16(jnp.concatenate([oa_s[slot, a // 2:b // 2, :] for a, b in cuts], axis=0))
        shared = _dot(wot_s[rows, 768:896], o((384, 448), (320, 384)))
        a = jnp.concatenate([_dot(wot_s[rows, 0:384], o((0, 384))) + shared,
                             _dot(wot_s[rows, 384:768], o((0, 320), (384, 448))) + shared], axis=0)
        g = jnp.broadcast_to(g_s[blk][0:1], (112, 128))
        rows = slice(112 * k, 112 * (k + 1))
        out_v[blk, rows, :] = (g * a + (1.0 - g) * bt_s[rows, :]).astype(BF16)

    def out_copy(blk):
        return pltpu.make_async_copy(out_v.at[blk], out_hbm.at[0, :, _rows(blk * 128, 128, 128)], osem)

    slabs = [list(range(5)) if t <= 1 else [0] + list(range(t, 5)) for t in range(5)]
    tiles = [(t, c) for t in range(5) for c in range(4) if c < 3 or t in (0, 1, 3)]
    slab = lambda y, i: y[8 * i:8 * (i + 1)]
    split = lambda y, t: {i: slab(y, n) for n, i in enumerate(slabs[t])}

    def accumulate(acc, y):
        for i, v in y.items():
            acc[i] = acc[i] + v if i in acc else v

    def step(qb, slot, hg, mem, order):
        s = qb * 4 + hg
        h = jnp.concatenate([mem, xn_s[_rows(s * 32, 32, 32), :]], axis=0)
        lo8 = _iota((8, 128), 1) < 64
        lo40 = _iota((40, 128), 1) < 64
        a12 = h[:, 256:384]
        a13 = jnp.where(lo40, a12, h[:, 384:512])
        a32 = jnp.where(lo40, h[:, 384:512], a12)
        early, scores, probs, outs, done = {}, [{} for _ in range(5)], [], [{} for _ in range(4)], set()
        new_mem, denom, heads = {}, {}, {}

        def early_passes(q, c):
            o = (q * 7 + c) * D
            w = lambda k: _to_bf16(ar2[o + 64 * k:o + 64 * (k + 1), :])
            shared = _dot(a32, w(6))
            early[q, c] = (_dot(h[:, 0:128], w(0)) + _dot(a12, w(2)) + shared,
                           _dot(h[:, 0:128], w(3)) + _dot(a13, w(5)) + shared)

        def two_tiles(w, q, c):
            o = (q * 7 + c) * D
            if w is ar2 and (q, c) in early:
                return (early[q, c][0] + _dot(h[:, 128:256], _to_bf16(w[o + 64:o + 128, :])),
                        early[q, c][1] + _dot(h[:, 128:256], _to_bf16(w[o + 256:o + 320, :])))
            shared = _dot(a32, _to_bf16(w[o + 384:o + 448, :]))
            return (_dot(h[:, 0:384], _to_bf16(w[o:o + 192, :])) + shared,
                    _dot(jnp.concatenate([h[:, 0:256], a13], axis=1), _to_bf16(w[o + 192:o + 384, :])) + shared)

        def project(w, dst, q, c):
            def put(t, c, i, uv):
                dst[t, c, 32 * q + 16 * i:32 * q + 16 * (i + 1), :] = jnp.concatenate(uv, axis=0).astype(BF16)

            if c < 2:
                for i in range(2):
                    y = two_tiles(w, q, 3 * i + c)
                    for t in range(5):
                        put(t, c, i, [slab(v, t) for v in y])
                return
            z = two_tiles(w, q, 6)
            put(0, 3, 0, [jnp.where(lo8, slab(v, 0), 0.0) for v in z])
            put(0, 3, 1, [jnp.where(lo8, 0.0, slab(v, 0)) for v in z])
            dz = {t: [slab(v, t + 1) - slab(v, t) for v in z] for t in (1, 3)}
            moved = {t: [pltpu.roll(jnp.where(lo8, d, slab(v, t)), 64, 1) for d, v in zip(dz[t], z)]
                     for t in (1, 3)}
            for i in range(2):
                y = two_tiles(w, q, 3 * i + 2)
                put(0, 2, i, [slab(v, 0) for v in y])
                for t in (1, 3):
                    hi = moved[t] if i == 0 else dz[t]
                    lo = [slab(v, t) for v in z] if i == 0 else moved[t]
                    put(t, 2, i, [jnp.where(lo8, slab(v, t), slab(v, t) - slab(v, t + 1)) for v in y])
                    put(t + 1, 2, i, [jnp.where(lo8, slab(v, t + 1), e) for v, e in zip(y, hi)])
                    put(t, 3, i, [jnp.where(lo8, e, slab(v, t + 1)) for v, e in zip(y, lo)])

        def scores_b(k):
            for t, c in tiles[4 * k:4 * k + 4]:
                lhs = h[:, 128 * c:128 * (c + 1)] if c < 2 or t == 0 else a32 if c == 3 else a12 if t % 2 else a13
                y = split(_dot(jnp.concatenate([slab(lhs, i) for i in slabs[t]], axis=0), ts_s[t, c], NT), t)
                accumulate(scores[t], y)
                if c == 3 and t:
                    accumulate(scores[t + 1], {i: y[i] for i in slabs[t + 1]})
            done.add(k)
            if len(done) < 5:
                return
            z = [{i: v * (256.0 ** -0.5 * LOG2E) for i, v in sc.items()} for sc in scores]
            causal = _iota((8, 128), 0) >= (_iota((8, 128), 1) & 7)
            for t in range(1, 5):
                z[t][t] = jnp.where(causal, z[t][t], NEG)
            over_keys = lambda op: _group8_allreduce(jnp.concatenate(
                [functools.reduce(op, [zt[i] for zt in z if i in zt]) for i in range(5)], axis=0), op)
            top = over_keys(jnp.maximum)
            z = [{i: jnp.exp2(v - slab(top, i)) for i, v in zt.items()} for zt in z]
            inv = 1.0 / over_keys(jnp.add)
            probs.extend({i: v * slab(inv, i) for i, v in zt.items()} for zt in z)

        def output_b(k):
            todo = ([(t, k) for t in range(5)] if k < 2 else
                    [(0, 2), (1, 2), (3, 2)] if k == 2 else [(0, 3), (1, 3), (2, 2), (3, 3), (4, 2)])
            for t, c in todo:
                p = probs[t]
                if c == 3 and t:
                    p = {i: v + probs[t + 1][i] if i in probs[t + 1] else v for i, v in p.items()}
                y = split(_dot(jnp.concatenate([p[i] for i in slabs[t]], axis=0), vs_s[t, c]), t)
                if c < 2 or t == 0 or (c == 2 and t % 2):
                    accumulate(outs[c], y)
                else:
                    accumulate(outs[5 - c], {i: jnp.where(lo8, 0.0, v) for i, v in y.items()})
                    accumulate(outs[c], {i: jnp.where(lo8, v, 0.0) for i, v in y.items()})
            done.add(("out", k))
            for c in ((k,) if k < 2 else (2, 3) if {("out", 2), ("out", 3)} <= done else ()):
                o = jnp.concatenate([outs[c][i] for i in range(5)], axis=0)
                if c == 3:
                    o = o + pltpu.roll(o, 64, 1)
                b_s[slot, 32 * hg:32 * (hg + 1), 128 * c:128 * (c + 1)] = o[8:40]
                new_mem[c] = o[0:8]

        def softmax_a(i):
            row = 2 * _iota((56, 128), 0)
            head = sum((row >= 28 * j).astype(jnp.int32) for j in (1, 2, 3))
            mine = ((head + i) & 3) == (_iota((56, 128), 1) >> 5)
            ones = _to_u32(jnp.where(_iota((16, 128), 0) == 15, 1.0, 0.0).astype(BF16))
            q = jnp.concatenate([jnp.where(mine, ar1[_rows(QT + s * 56, 56, 8), :], jnp.uint32(0)), ones], axis=0)
            k0 = KA + 1152 * hg + qb * 64 + 16 * i
            cuts = (0, 40, 72, 112, 144) if i % 2 == 0 else (0, 32, 72, 104, 144)
            z = jnp.concatenate([_dot(_to_bf16(ar1[_rows(k0 + a, b - a, 8), :]), _to_bf16(q))
                                 for a, b in zip(cuts[:-1], cuts[1:])], axis=0)
            newest = _iota((32, 128), 0) <= (_iota((32, 128), 1) & 31)
            z = jnp.concatenate([jnp.where(newest, z[256:288], z[0:32]), z[32:256]], axis=0)
            p = jnp.exp2(z - jnp.max(z, axis=0, keepdims=True))
            denom[i] = jnp.broadcast_to(jnp.sum(p, axis=0, keepdims=True), (8, 128))
            pz_s[i] = _to_u32(jnp.concatenate([
                jnp.where(newest, 0.0, p[0:32]), p[32:256], jnp.where(newest, p[0:32], 0.0)], axis=0).astype(BF16))

        def regroup_a(part):
            if part == 0:
                denom["inv"] = _regroup([1.0 / denom[i] for i in range(4)])
            for r in range(3 * part, 3 * part + 3):
                z = [pz_s[i, 16 * (r - i):16 * (r - i + 1), :] if 0 <= r - i <= 8 else jnp.zeros((16, 128), U32)
                     for i in range(4)]
                for j, v in enumerate(_regroup(z)):
                    pa_s[j, 16 * r:16 * (r + 1), :] = v

        def output_a(j):
            v = jnp.concatenate([ar1[_rows(VT + 2016 * hg + (qb + i) * 112 + HEAD_WIN[j], 32, 8), :]
                                 for i in range(3)], axis=1)
            o = _dot(pltpu.bitcast(v, F32), _to_bf16(pa_s[j])) * jnp.concatenate([denom["inv"][j]] * 4, axis=0)
            heads[j] = pltpu.roll(o, 128 - 32 * j, 1) if j else o
            if len(heads) == 4:
                oa_s[slot, 56 * hg:56 * (hg + 1), :] = _to_u32(
                    _join_heads([heads[i] for i in range(4)]).astype(BF16))

        pieces = dict(
            e=early_passes, t=functools.partial(project, ar2, ts_s), v=functools.partial(project, ar3, vs_s),
            sb=scores_b, pb=output_b, sa=softmax_a, rg=regroup_a, pa=output_a,
            tr=lambda: transpose_b(1 - slot, hg),
            fin=lambda: finalize(1 - slot, hg, jnp.maximum(qb - 1, 0)))
        for name in order.split():
            kind = name.rstrip("0123456789")
            pieces[kind](*map(int, name[len(kind):]))
        return jnp.concatenate([new_mem[c] for c in range(4)], axis=1)

    def blocks(i, mem):
        for u in range(NB):
            @pl.when(i * NB + u - NB - 1 >= 0)
            def _():
                out_copy(i * NB + u - NB - 1).start()

        orders = [o for o in ORDER.split("|") if o]
        for u in range(NB):
            for hg in range(4):
                mem = step(i * NB + u, u % 2, hg, mem, orders[(4 * u + hg) % len(orders)])
        return mem

    m0 = mem0_v[...].astype(F32)
    lax.fori_loop(0, NQB // NB, blocks, jnp.concatenate([m0, m0[:, 384:448]], axis=1))

    for blk in range(NQB - NB - 1, NQB - 1):
        out_copy(blk).start()
    for k in range(4):
        transpose_b(1, k)
    for k in range(4):
        finalize(1, k, NQB - 1)
    out_copy(NQB - 1).start()
    for blk in range(NQB):
        out_copy(blk).wait()


@functools.partial(jax.jit, static_argnames=("B_seg_len",))
def pallas_gated_mix__sliding_block__memory_aug_recurrent_mem_tr__prompt_kernel(
        A_x, A_wqkv, A_wo, B_x, B_mem0, B_Wq, B_Wk, B_Wv, B_Wo, B_seg_len, gate_w):
    del B_x
    assert A_x.shape == (1, S, D) and B_Wq.shape == (D, 16, 256)
    assert B_mem0.shape == (1, 8, D) and B_seg_len == 32
    flat = lambda w: w.reshape(D * 16, 256)
    hbm = pl.BlockSpec(memory_space=pltpu.HBM)
    vmem = pltpu.VMEM
    out_t = pl.pallas_call(
        _kernel,
        out_shape=jax.ShapeDtypeStruct((1, D, S), BF16),
        in_specs=[hbm] * 9,
        out_specs=hbm,
        scratch_shapes=[
            vmem((D, S), BF16), vmem((D, 3 * D), BF16), vmem((D, D), BF16), vmem((8, D), BF16), vmem((D,), BF16),
            vmem((D * 16, 256), BF16), vmem((D * 16, 256), BF16), vmem((D * 16, 256), BF16),
            vmem((16, D, 256), BF16),
            vmem((30592, 128), U32), vmem((19712, 128), U32), vmem((12544, 128), U32),
            vmem((336, 896), U32), vmem((672, 256), U32), vmem((D, 512), F32), vmem((8, D), F32),
            vmem((224, 896), F32), vmem((S, 512), F32), vmem((NQB, 8, 128), F32),
            vmem((2, 224, 128), U32), vmem((2, 128, 512), F32), vmem((512, 128), F32), vmem((NQB, D, 128), BF16),
            vmem((5, 4, 128, 128), BF16), vmem((5, 4, 128, 128), BF16),
            vmem((4, 192, 128), U32), vmem((4, 144, 128), U32),
            pltpu.SemaphoreType.DMA((25,)), pltpu.SemaphoreType.DMA(()),
        ],
        compiler_params=pltpu.CompilerParams(vmem_limit_bytes=100 * 2**20),
        name="gated_mix_attention",
    )(A_x.transpose(0, 2, 1), A_wqkv, A_wo, B_mem0, flat(B_Wq), flat(B_Wk), flat(B_Wv),
      B_Wo.transpose(0, 2, 1), gate_w)
    return out_t.transpose(0, 2, 1)
```
